```python
import jax
import jax.numpy as jnp

def _softmax(x, axis=-1):
    return jax.nn.softmax(x, axis=axis)

def _gelu(x):
    return jax.nn.gelu(x, approximate=True)

def _silu(x):
    return jax.nn.silu(x)

def _sigmoid(x):
    return jax.nn.sigmoid(x)

def _layernorm(x, axis=-1, eps=1e-05):
    m = jnp.mean(x, axis=axis, keepdims=True)
    v = jnp.var(x, axis=axis, keepdims=True)
    return (x - m) / jnp.sqrt(v + eps)

def _scatter_add(tgt, idx, src, axis=0):
    return tgt.at[idx].add(src)

def _segment_sum(src, seg, n):
    return jax.ops.segment_sum(src, seg, n)

class _Rng:

    def __init__(self, key):
        self._k = key

    def _next(self):
        self._k, sub = jax.random.split(self._k)
        return sub

    def normal(self, shape):
        return jax.random.normal(self._next(), shape, dtype=jnp.bfloat16)

    def randint(self, lo, hi, shape):
        return jax.random.randint(self._next(), shape, lo, hi, dtype=jnp.int32)

    def uniform(self, shape, lo=0.0, hi=1.0):
        return jax.random.uniform(self._next(), shape, jnp.bfloat16, lo, hi)

    def permutation(self, n):
        return jax.random.permutation(self._next(), n)
kernel_name = 'adaLN_cond__memory_aug_recurrent_mem_tr__mixer_s_mlp__prompt'

def setup_inputs():
    _rng = _Rng(jax.random.key(int.from_bytes(__import__("os").urandom(4), "little")))
    _w = lambda a: (lambda t: t.astype(jnp.bfloat16) if jnp.issubdtype(t.dtype, jnp.floating) else t)(jnp.asarray(a))

    def _A_setup():
        B, S, Dm = (1, 2048, 1024)
        H, Dh = (32, 128)
        M, seg = (8, 32)
        seg = min(seg, S)
        S = S // seg * seg
        return {'x': _w((lambda *s: _rng.normal(s) * 0.05)(B, S, Dm)), 'mem0': _w((lambda *s: _rng.normal(s) * 0.05)(B, M, Dm)), 'Wq': _w((lambda *s: _rng.normal(s) * 0.05)(Dm, H, Dh) * Dm ** (-0.5)), 'Wk': _w((lambda *s: _rng.normal(s) * 0.05)(Dm, H, Dh) * Dm ** (-0.5)), 'Wv': _w((lambda *s: _rng.normal(s) * 0.05)(Dm, H, Dh) * Dm ** (-0.5)), 'Wo': _w((lambda *s: _rng.normal(s) * 0.05)(H, Dh, Dm) * (H * Dh) ** (-0.5)), 'seg_len': seg}
    _A_in = _A_setup()

    def _B_setup():
        B, S, D, F = (1, 2048, 1024, 3584)
        return {'x': _w((lambda *s: _rng.normal(s) * 0.05)(B, S, D)), 'w1': _w((lambda *s: _rng.normal(s) * 0.05)(D, D) * D ** (-0.5)), 'w2': _w((lambda *s: _rng.normal(s) * 0.05)(D, D) * D ** (-0.5)), 'w3': _w((lambda *s: _rng.normal(s) * 0.05)(D, F) * D ** (-0.5)), 'w4': _w((lambda *s: _rng.normal(s) * 0.05)(F, D) * F ** (-0.5))}
    _B_in = _B_setup()
    return {'A_x': _A_in['x'], 'A_mem0': _A_in['mem0'], 'A_Wq': _A_in['Wq'], 'A_Wk': _A_in['Wk'], 'A_Wv': _A_in['Wv'], 'A_Wo': _A_in['Wo'], 'A_seg_len': _A_in['seg_len'], 'B_x': _B_in['x'], 'B_w1': _B_in['w1'], 'B_w2': _B_in['w2'], 'B_w3': _B_in['w3'], 'B_w4': _B_in['w4'], 'c': _w((lambda *s: _rng.normal(s) * 0.05)(1, 1024)), 'w_mod': _w((lambda *s: _rng.normal(s) * 0.05)(1024, 6 * 1024) * 1024 ** (-0.5))}

def reference(A_x, A_mem0, A_Wq, A_Wk, A_Wv, A_Wo, A_seg_len, B_x, B_w1, B_w2, B_w3, B_w4, c, w_mod):

    def _A_ref(x, mem0, Wq, Wk, Wv, Wo, seg_len):
        B, S, Dm = x.shape
        H, Dh = (Wq.shape[1], Wq.shape[2])
        M = mem0.shape[1]
        scale = Dh ** (-0.5)
        n_seg = S // seg_len
        L = M + seg_len
        idx = jnp.arange(L)
        mask = (idx[:, None] < M) | (idx[:, None] >= idx[None, :])
        mem = mem0
        outs = []
        for s in range(n_seg):
            xs = x[:, s * seg_len:(s + 1) * seg_len, :].copy()
            h = jnp.concatenate([mem, xs], axis=1)
            q = jnp.einsum('btd,dhe->bhte', h, Wq)
            k = jnp.einsum('btd,dhe->bhte', h, Wk)
            v = jnp.einsum('btd,dhe->bhte', h, Wv)
            scores = jnp.einsum('bhqe,bhke->bhqk', q, k) * scale
            scores = jnp.where(mask[None, None], scores, -1000000000.0)
            p = _softmax(scores, axis=-1)
            o = jnp.einsum('bhqk,bhke->bhqe', p, v)
            o = jnp.einsum('bhte,hed->btd', o, Wo)
            mem = o[:, :M, :].copy()
            outs.append(o[:, M:, :])
        return jnp.concatenate(outs, axis=1)

    def _B_ref(x, w1, w2, w3, w4):
        B, S, D = x.shape
        h = _gelu(_layernorm(x, axis=-1) @ w1)
        c = D // 4
        g0 = jnp.pad(h[:, :, 0 * c:1 * c], ((0, 0), (1, 0), (0, 0)))[:, :S, :]
        g1 = jnp.pad(h[:, :, 1 * c:2 * c], ((0, 0), (0, 1), (0, 0)))[:, 1:, :]
        g2 = jnp.pad(h[:, :, 2 * c:3 * c], ((0, 0), (2, 0), (0, 0)))[:, :S, :]
        g3 = jnp.pad(h[:, :, 3 * c:], ((0, 0), (0, 2), (0, 0)))[:, 2:, :]
        hs = jnp.concatenate([g0, g1, g2, g3], axis=-1) @ w2
        x1 = x + hs
        h2 = _gelu(_layernorm(x1, axis=-1) @ w3) @ w4
        return x1 + h2
    x = A_x
    mod = (_silu(c) @ w_mod).reshape(c.shape[0], 6, 1, -1)
    sa, ca, ga, sb, cb, gb = (mod[:, 0].copy(), mod[:, 1].copy(), mod[:, 2].copy(), mod[:, 3].copy(), mod[:, 4].copy(), mod[:, 5].copy())
    h = _layernorm(x, axis=-1) * (1 + ca) + sa
    x = x + ga * _A_ref(h, A_mem0, A_Wq, A_Wk, A_Wv, A_Wo, A_seg_len)
    h = _layernorm(x, axis=-1) * (1 + cb) + sb
    x = x + gb * _B_ref(h, B_w1, B_w2, B_w3, B_w4)
    return x
```

```python
import math

import jax
import jax.numpy as jnp
from jax import lax
import jax.experimental.pallas as pl
import jax.experimental.pallas.tpu as pltpu

F32, BF16, U32 = jnp.float32, jnp.bfloat16, jnp.uint32

SEG = 32
TAIL = 8
BODY = SEG - TAIL
OCT = 8
NSTAGE = 4
RB = 512
FC = 512
HALO = 8
EPS = 1e-5


def _layernorm(x):
    m = jnp.mean(x, axis=-1, keepdims=True)
    d = x - m
    v = jnp.mean(d * d, axis=-1, keepdims=True)
    return d * lax.rsqrt(v + EPS)


def _gelu(x):
    c1 = math.sqrt(2.0 / math.pi)
    hx = 0.5 * x
    return hx + hx * jnp.tanh(x * (c1 + (c1 * 0.044715) * (x * x)))


def _dot(a, b):
    return jnp.dot(a, b, preferred_element_type=F32)


def _packed(ref_value):
    return pltpu.bitcast(ref_value, BF16)


def _kernel(x_hbm, mem_hbm, wq_hbm, wk_hbm, wv_hbm, wo_hbm, w1_hbm, w2_hbm, w3_hbm, w4_hbm,
            c_hbm, wmod_hbm, out_hbm,
            x_v, act, big, w1_v, w2_v, w3_v, w4_v, c_v, mem_v, mod, sem):
    NSEG, _, D = x_hbm.shape
    _, H, DH = wq_hbm.shape
    M = mem_hbm.shape[0]
    S = NSEG * SEG
    F = w3_hbm.shape[1]
    NO = H // OCT
    ROWS = M + BODY
    NT = NSEG * TAIL
    scale = DH ** -0.5

    def copy(src, dst, i):
        return pltpu.make_async_copy(src, dst, sem.at[i])

    cp_c = copy(c_hbm, c_v, 0)
    cp_mem = copy(mem_hbm, mem_v, 1)
    cp_xt = copy(x_hbm.at[:, pl.ds(BODY, TAIL), :], x_v.at[:, pl.ds(BODY, TAIL), :], 2)
    cp_xb = copy(x_hbm.at[:, pl.ds(0, BODY), :], x_v.at[:, pl.ds(0, BODY), :], 3)
    cp_w = [copy(w1_hbm, w1_v, 4), copy(w2_hbm, w2_v, 5), copy(w3_hbm, w3_v, 6),
            copy(w4_hbm, w4_v, 7)]

    def cp_mod(j, slot):
        return copy(wmod_hbm.at[:, pl.ds(j * D, D)], big.at[slot], 8 + slot)

    def cp_wo(j):
        return copy(wo_hbm.at[pl.ds(j * D, D), :], big.at[j], 8 + j)

    def modulation(j, slot):
        c = c_v[...].astype(F32)
        sc = jnp.broadcast_to(c * jax.nn.sigmoid(c), (16, D)).astype(BF16)
        mod[j] = _dot(sc, big[slot])[:8]

    def attention(stage, wqkv, wo, ht, pre, otail, fill, wsem):
        def cp_oct(w_hbm, o, slot):
            return pltpu.make_async_copy(
                w_hbm.at[:, pl.ds(pl.multiple_of(o * OCT, OCT), OCT), :], stage.at[slot],
                wsem.at[slot])

        def start_oct(i):
            for m, w_hbm in enumerate((wq_hbm, wk_hbm, wv_hbm)):
                @pl.when(i // NO == m)
                def _():
                    cp_oct(w_hbm, i % NO, i % NSTAGE).start()

        def relayout(i):
            n = 128
            for b in range(D // n):
                w = stage[i % NSTAGE, pl.ds(b * n, n), :, :].reshape(n * OCT, DH)
                w = pltpu.bitcast(w, U32).reshape(n // 2, OCT, DH)
                w = jnp.swapaxes(w, 0, 1)
                for j in range(OCT // 2):
                    even, odd = w[j], w[OCT // 2 + j]
                    rows = pl.ds(b * (n // 2), n // 2)
                    wqkv[i, rows, pl.ds(2 * j * DH, DH)] = (even & 0xFFFF) | (odd << 16)
                    wqkv[i, rows, pl.ds((2 * j + 1) * DH, DH)] = (even >> 16) | ((odd >> 16) << 16)

        def project_tail(i):
            lhs = _packed(ht[...])
            for j in range(OCT // 2):
                r = _dot(lhs, _packed(wqkv[i, :, pl.ds(2 * j * DH, 2 * DH)]))
                r = jnp.concatenate([r[:, :DH].reshape(NSEG, TAIL, DH),
                                     r[:, DH:].reshape(NSEG, TAIL, DH)], axis=1)
                r = r.reshape(2 * NT, DH).astype(BF16)
                pre[i, :, pl.ds(j * DH, DH)] = pltpu.bitcast(r, U32)

        cp_c.start()
        cp_mod(0, 0).start()
        cp_mod(1, 1).start()
        cp_xt.start()
        cp_mem.start()
        cp_oct(wq_hbm, 0, 0).start()

        def head_pos(i):
            head = jnp.where(i < 2 * ROWS, i // ROWS, (i - 2 * ROWS) // TAIL)
            pos = jnp.where(i < 2 * ROWS, i % ROWS, ROWS + i % TAIL)
            return head, pos

        hr, pr = head_pos(lax.broadcasted_iota(jnp.int32, fill.shape, 0))
        hc, pc = head_pos(lax.broadcasted_iota(jnp.int32, fill.shape, 1))
        visible = (pr < M) | (pr >= pc)
        fill[...] = jnp.where(hr == hc, jnp.where(visible, 0.0, -1e9 / scale), -jnp.inf)

        cp_c.wait()
        cp_mod(0, 0).wait()
        modulation(0, 0)
        cp_mod(1, 1).wait()
        for i in range(1, NSTAGE):
            cp_oct(wq_hbm, i, i).start()
        modulation(1, 1)
        shift, gain = mod[0][:1], 1.0 + mod[1][:1]
        cp_xt.wait()
        xt = x_v[:, pl.ds(BODY, TAIL), :].astype(F32).reshape(NT, D)
        ht[...] = pltpu.bitcast((_layernorm(xt) * gain + shift).astype(BF16), U32)
        cp_oct(wq_hbm, 0, 0).wait()
        relayout(0)
        cp_xb.start()
        for j in range(4):
            cp_wo(j).start()

        def tail_step(i, carry):
            @pl.when(i + NSTAGE < 3 * NO)
            def _():
                start_oct(i + NSTAGE)
            cp_oct(wq_hbm, 0, (i + 1) % NSTAGE).wait()
            project_tail(i)
            relayout(i + 1)
            return carry

        lax.fori_loop(0, 3 * NO - 1, tail_step, 0)
        cp_xb.wait()
        cp_mem.wait()
        for j in range(4):
            cp_wo(j).wait()
        project_tail(3 * NO - 1)
        for j in range(4):
            wo[pl.ds(j * (D // 2), D // 2), :] = pltpu.bitcast(big[j], U32)

        def norm_body(i, carry):
            segs = pl.ds(i * 8, 8)
            xb = x_v[segs, pl.ds(0, BODY), :].astype(F32).reshape(8 * BODY, D)
            act[segs, pl.ds(0, BODY), :] = (_layernorm(xb) * gain + shift).reshape(8, BODY, D)
            return carry

        lax.fori_loop(0, NSEG // 8, norm_body, 0)
        for j in range(4):
            cp_mod(2 + j, j).start()
        for cp in cp_w:
            cp.start()

        def segment(s, mem):
            lhs = jnp.concatenate([mem, act[s, pl.ds(0, BODY), :]], axis=0).astype(BF16)
            tail = pl.ds(pl.multiple_of(s * TAIL, TAIL), TAIL)
            pad = jnp.zeros((fill.shape[1] - fill.shape[0], DH), BF16)
            heads = []
            for p in range(H // 2):
                o, j = divmod(p, OCT // 2)

                def project(m, *extra):
                    r = _dot(lhs, _packed(wqkv[m * NO + o, :, pl.ds(2 * j * DH, 2 * DH)]))
                    r = r.astype(BF16)
                    t = _packed(pre[m * NO + o, tail, pl.ds(j * DH, DH)])
                    return jnp.concatenate([r[:, :DH], r[:, DH:], t, *extra], axis=0)

                q, k, v = project(0), project(1, pad), project(2, pad)
                sc = lax.dot_general(q, k, (((1,), (1,)), ((), ())), preferred_element_type=F32)
                f = fill[...]
                sc = jnp.where(f == 0.0, sc, f)
                e = jnp.exp2((sc - jnp.max(sc, axis=-1, keepdims=True))
                             * (scale * math.log2(math.e)))
                ov = _dot(e.astype(BF16), v) * (1.0 / jnp.sum(e, axis=-1, keepdims=True))
                heads += [ov[:ROWS].astype(BF16), ov[ROWS:2 * ROWS].astype(BF16)]
                otail[tail, pl.ds(2 * p * DH, DH)] = ov[2 * ROWS:2 * ROWS + TAIL]
                otail[tail, pl.ds((2 * p + 1) * DH, DH)] = ov[2 * ROWS + TAIL:]
            a = _dot(jnp.concatenate(heads, axis=1), _packed(wo[...]))
            act[s, pl.ds(0, BODY), :] = a[M:]
            return a[:M]

        lax.fori_loop(0, NSEG, segment, mem_v[...].astype(F32))

        a = _dot(otail[...].astype(BF16), _packed(wo[...]))
        act[:, pl.ds(BODY, TAIL), :] = a.reshape(NSEG, TAIL, D)

    pl.run_scoped(
        attention,
        pltpu.VMEM((NSTAGE, D, OCT, DH), BF16),
        pltpu.VMEM((3 * NO, D // 2, OCT * DH), U32),
        pltpu.VMEM((H * DH // 2, D), U32),
        pltpu.VMEM((NT // 2, D), U32),
        pltpu.VMEM((3 * NO, NT, OCT * DH // 2), U32),
        pltpu.VMEM((NT, H * DH), F32),
        pltpu.VMEM((2 * (M + SEG), 128), F32),
        pltpu.SemaphoreType.DMA((NSTAGE,)),
    )

    def mixer(hb, hh, ostage, osem):
        for j in range(4):
            cp_mod(2 + j, j).wait()
            modulation(2 + j, j)
        for cp in cp_w:
            cp.wait()
        gate_a, shift, gain, gate_b = mod[2][:1], mod[3][:1], 1.0 + mod[4][:1], mod[5][:1]
        nseg = RB // SEG
        hh[pl.ds(0, HALO), :] = jnp.zeros((HALO, D), F32)
        hh[pl.ds(HALO + S, HALO), :] = jnp.zeros((HALO, D), F32)

        def token_mlp(i, carry):
            segs = pl.ds(i * nseg, nseg)
            r0 = pl.multiple_of(i * RB, RB)
            x = x_v[segs].astype(F32).reshape(RB, D) + gate_a * act[segs].reshape(RB, D)
            act[segs] = x.reshape(nseg, SEG, D)
            h = _layernorm(x) * gain + shift
            hb[pl.ds(r0, RB), :] = h
            hh[pl.ds(HALO + r0, RB), :] = _gelu(_dot(_layernorm(h).astype(BF16), w1_v[...]))
            return carry

        lax.fori_loop(0, S // RB, token_mlp, 0)

        def cp_out(i):
            return pltpu.make_async_copy(
                ostage.at[i % 2], out_hbm.at[pl.ds(pl.multiple_of(i * RB, RB), RB), :],
                osem.at[i % 2])

        def channel_mlp(i, carry):
            segs = pl.ds(i * nseg, nseg)
            r0 = pl.multiple_of(i * RB, RB)
            g = D // 4
            shifted = [hh[pl.ds(r0, RB + 2 * HALO), pl.ds(n * g, g)][HALO + d:HALO + d + RB]
                       for n, d in enumerate((-1, 1, -2, 2))]
            x1 = hb[pl.ds(r0, RB), :] + _dot(
                jnp.concatenate(shifted, axis=1).astype(BF16), w2_v[...])
            z = _layernorm(x1).astype(BF16)
            y = x1
            for f in range(F // FC):
                u = _gelu(_dot(z, w3_v[:, pl.ds(f * FC, FC)])).astype(BF16)
                y = y + _dot(u, w4_v[pl.ds(f * FC, FC), :])

            @pl.when(i >= 2)
            def _():
                cp_out(i - 2).wait()

            ostage[i % 2] = (act[segs].reshape(RB, D) + gate_b * y).astype(BF16)
            cp_out(i).start()
            return carry

        lax.fori_loop(0, S // RB, channel_mlp, 0)
        cp_out(S // RB - 2).wait()
        cp_out(S // RB - 1).wait()

    pl.run_scoped(
        mixer,
        pltpu.VMEM((S, D), F32),
        pltpu.VMEM((S + 2 * HALO, D), F32),
        pltpu.VMEM((2, RB, D), BF16),
        pltpu.SemaphoreType.DMA((2,)),
    )


@jax.jit
def pallas_adaLN_cond__memory_aug_recurrent_mem_tr__mixer_s_mlp__prompt_kernel(
    A_x: jax.Array,
    A_mem0: jax.Array,
    A_Wq: jax.Array,
    A_Wk: jax.Array,
    A_Wv: jax.Array,
    A_Wo: jax.Array,
    A_seg_len: jax.Array,
    B_x: jax.Array,
    B_w1: jax.Array,
    B_w2: jax.Array,
    B_w3: jax.Array,
    B_w4: jax.Array,
    c: jax.Array,
    w_mod: jax.Array,
):
    del A_seg_len, B_x
    B, S, D = A_x.shape
    M = A_mem0.shape[1]
    _, H, DH = A_Wq.shape
    F = B_w3.shape[1]
    assert B == 1 and M == 8 and DH == 128 and H * DH == 4 * D and S % RB == 0 and F % FC == 0

    out = pl.pallas_call(
        _kernel,
        out_shape=jax.ShapeDtypeStruct((S, D), A_x.dtype),
        in_specs=[pl.BlockSpec(memory_space=pl.ANY)] * 12,
        out_specs=pl.BlockSpec(memory_space=pl.ANY),
        scratch_shapes=[
            pltpu.VMEM((S // SEG, SEG, D), BF16),
            pltpu.VMEM((S // SEG, SEG, D), F32),
            pltpu.VMEM((4, D, D), BF16),
            pltpu.VMEM((D, D), BF16),
            pltpu.VMEM((D, D), BF16),
            pltpu.VMEM((D, F), BF16),
            pltpu.VMEM((F, D), BF16),
            pltpu.VMEM((1, D), BF16),
            pltpu.VMEM((M, D), BF16),
            pltpu.VMEM((6, 8, D), F32),
            pltpu.SemaphoreType.DMA((12,)),
        ],
        compiler_params=pltpu.CompilerParams(vmem_limit_bytes=124 * 2**20),
    )(A_x.reshape(S // SEG, SEG, D), A_mem0.reshape(M, D), A_Wq, A_Wk, A_Wv,
      A_Wo.reshape(H * DH, D), B_w1, B_w2, B_w3, B_w4, c, w_mod)
    return out.reshape(B, S, D)
```

```python
import math

import jax
import jax.numpy as jnp
from jax import lax
import jax.experimental.pallas as pl
import jax.experimental.pallas.tpu as pltpu

F32, BF16, U32 = jnp.float32, jnp.bfloat16, jnp.uint32

SEG = 32
TAIL = 8
BODY = SEG - TAIL
OCT = 8
LANES = 128
NSTAGE = 4
SB = 16
RB2 = 512
RB = 128
FC = 512
TG = 4
EPS = 1e-5


def _layernorm(x):
    m = jnp.mean(x, axis=-1, keepdims=True)
    d = x - m
    v = jnp.mean(d * d, axis=-1, keepdims=True)
    return d * lax.rsqrt(v + EPS)


def _gelu(x):
    c1 = math.sqrt(2.0 / math.pi)
    hx = 0.5 * x
    return hx + hx * jnp.tanh(x * (c1 + (c1 * 0.044715) * (x * x)))


def _dot(a, b):
    return jnp.dot(a, b, preferred_element_type=F32)


def _packed(words):
    return pltpu.bitcast(words, BF16)


def _kernel(x_hbm, mem_hbm, wq_hbm, wk_hbm, wv_hbm, wo_hbm, w1_hbm, w2_hbm, w3_hbm, w4_hbm,
            c_hbm, wmod_hbm, out_hbm,
            x_v, act, otail, wmod_v, wo_v, w1_v, w2_v, w3_v, w4_v, c_v, mem_v, mod, sem):
    NSEG, _, D = x_hbm.shape
    _, H, DH = wq_hbm.shape
    M = mem_hbm.shape[0]
    S = NSEG * SEG
    F = w3_hbm.shape[1]
    NO = H // OCT
    ROWS = M + BODY
    NT = NSEG * TAIL
    scale = DH ** -0.5
    body, tail = pl.ds(0, BODY), pl.ds(BODY, TAIL)

    def copy(src, dst, i):
        return pltpu.make_async_copy(src, dst, sem.at[i])

    cp_c = copy(c_hbm, c_v, 0)
    cp_mem = copy(mem_hbm, mem_v, 1)
    cp_xt = copy(x_hbm.at[:, tail, :], x_v.at[:, tail, :], 2)
    cp_xb = copy(x_hbm.at[:, body, :], x_v.at[:, body, :], 3)
    cp_w = [copy(w1_hbm, w1_v, 4), copy(w2_hbm, w2_v, 5), copy(w3_hbm, w3_v, 6),
            copy(w4_hbm, w4_v, 7)]
    cp_wo = [copy(wo_hbm.at[:, pl.ds(n * LANES, LANES)], wo_v.at[n], 12 + n)
             for n in range(D // LANES)]

    def cp_mod(j, slot):
        return copy(wmod_hbm.at[:, pl.ds(pl.multiple_of(j * D, D), D)], wmod_v.at[slot], 8 + slot)

    def modulation(j, slot):
        c = c_v[...].astype(F32)
        sc = jnp.broadcast_to(c * jax.nn.sigmoid(c), (16, D)).astype(BF16)
        mod[j] = _dot(sc, wmod_v[slot])[:8]

    def wo_rows(r0, n):
        return jnp.concatenate([wo_v[j, pl.ds(r0, n), :] for j in range(D // LANES)], axis=1)

    def attention(stage, wqkv, ht, pre, fill, wsem):
        def cp_oct(w_hbm, o, slot):
            return pltpu.make_async_copy(
                w_hbm.at[:, pl.ds(pl.multiple_of(o * OCT, OCT), OCT), :], stage.at[slot],
                wsem.at[slot])

        def relayout(i, b, n):
            w = stage[i % NSTAGE, pl.ds(pl.multiple_of(b * n, n), n), :, :].reshape(n * OCT, DH)
            w = jnp.swapaxes(pltpu.bitcast(w, U32).reshape(n // 2, OCT, DH), 0, 1)
            rows = pl.ds(pl.multiple_of(b * (n // 2), n // 2), n // 2)
            for j in range(OCT // 2):
                even, odd = w[j], w[OCT // 2 + j]
                wqkv[i, rows, pl.ds(2 * j * DH, DH)] = (even & 0xFFFF) | (odd << 16)
                wqkv[i, rows, pl.ds((2 * j + 1) * DH, DH)] = (even >> 16) | ((odd >> 16) << 16)

        cp_oct(wq_hbm, 0, 0).start()
        cp_xt.start()
        cp_c.start()
        cp_mem.start()

        def head_pos(i):
            head = jnp.where(i < 2 * ROWS, i // ROWS, (i - 2 * ROWS) // TAIL)
            pos = jnp.where(i < 2 * ROWS, i % ROWS, ROWS + i % TAIL)
            return head, pos

        hr, pr = head_pos(lax.broadcasted_iota(jnp.int32, fill.shape, 0))
        hc, pc = head_pos(lax.broadcasted_iota(jnp.int32, fill.shape, 1))
        visible = (pr < M) | (pr >= pc)
        fill[...] = jnp.where(hr == hc, jnp.where(visible, 0.0, -1e9 / scale), -jnp.inf)

        def first_relayout(b, carry):
            relayout(0, b, D // OCT)
            return carry

        def norm_tail(i, carry):
            segs = pl.ds(i * 8, 8)
            xt = x_v[segs, tail, :].astype(F32).reshape(8 * TAIL, D)
            act[segs, tail, :] = _layernorm(xt).reshape(8, TAIL, D)
            return carry

        def first_modulation(j, carry):
            cp_mod(j, j).wait()
            cp_oct(wq_hbm, j + 1, j + 1).start()
            modulation(j, j)
            return carry

        cp_xt.wait()
        cp_mod(0, 0).start()
        lax.fori_loop(0, NSEG // 8, norm_tail, 0)
        cp_oct(wq_hbm, 0, 0).wait()
        cp_mod(1, 1).start()
        lax.fori_loop(0, OCT, first_relayout, 0)
        cp_c.wait()
        lax.fori_loop(0, 2, first_modulation, 0)
        cp_oct(wq_hbm, 3, 3).start()
        shift, gain = mod[0][:1], 1.0 + mod[1][:1]
        ht[...] = pltpu.bitcast((act[:, tail, :].reshape(NT, D) * gain + shift).astype(BF16), U32)

        def project_tail(i, carry):
            for m, w_hbm in enumerate((wq_hbm, wk_hbm, wv_hbm)):
                @pl.when((i + NSTAGE) // NO == m)
                def _():
                    cp_oct(w_hbm, (i + NSTAGE) % NO, i % NSTAGE).start()

            @pl.when(i == NO)
            def _():
                cp_xb.start()

            @pl.when(i == 3 * NO - NSTAGE)
            def _():
                for cp in cp_wo:
                    cp.start()

            @pl.when(i + 1 < 3 * NO)
            def _():
                cp_oct(wq_hbm, 0, (i + 1) % NSTAGE).wait()

            nxt = jnp.minimum(i + 1, 3 * NO - 1)
            n = NT // TG
            for j in range(OCT // 2):
                for g in range(TG):
                    lhs = _packed(ht[pl.ds(g * n // 2, n // 2), :])
                    halves = []
                    for h in (2 * j, 2 * j + 1):
                        r = _dot(lhs, _packed(wqkv[i, :, pl.ds(h * DH, DH)]))
                        halves.append(r.reshape(n // TAIL, TAIL, DH))
                        relayout(nxt, h * TG + g, D // (OCT * TG))
                    r = jnp.concatenate(halves, axis=1).reshape(2 * n, DH).astype(BF16)
                    pre[i, pl.ds(g * n, n), pl.ds(j * DH, DH)] = pltpu.bitcast(r, U32)
            return carry

        lax.fori_loop(0, 3 * NO, project_tail, 0)

        def norm_body(s):
            act[s, body, :] = _layernorm(x_v[s, body, :].astype(F32)) * gain + shift

        cp_xb.wait()
        cp_mem.wait()
        for cp in cp_wo:
            cp.wait()
        norm_body(0)
        for j in range(4):
            cp_mod(2 + j, j).start()
        for cp in cp_w:
            cp.start()

        def segment(s, mem):
            lhs = jnp.concatenate([mem, act[s, body, :]], axis=0).astype(BF16)
            rows = pl.ds(pl.multiple_of(s * TAIL, TAIL), TAIL)
            pad = jnp.zeros((fill.shape[1] - fill.shape[0], DH), BF16)
            qkv, probs, heads = {}, {}, {}

            def project(p, m):
                o, j = divmod(p, OCT // 2)
                r = _dot(lhs, _packed(wqkv[m * NO + o, :, pl.ds(2 * j * DH, 2 * DH)]))
                r = r.astype(BF16)
                t = _packed(pre[m * NO + o, rows, pl.ds(j * DH, DH)])
                qkv[p, m] = [r[:, :DH], r[:, DH:], t]

            def scores(p):
                q = jnp.concatenate(qkv[p, 0], axis=0)
                k = jnp.concatenate(qkv[p, 1] + [pad], axis=0)
                sc = lax.dot_general(q, k, (((1,), (1,)), ((), ())), preferred_element_type=F32)
                f = fill[...]
                sc = jnp.where(f == 0.0, sc, f)
                e = jnp.exp2((sc - jnp.max(sc, axis=-1, keepdims=True))
                             * (scale * math.log2(math.e)))
                inv = pltpu.reciprocal(jnp.sum(e, axis=-1, keepdims=True), full_range=False)
                probs[p] = (e * inv).astype(BF16)

            def values(p, pad):
                ov = _dot(probs[p], jnp.concatenate(qkv[p, 2] + [pad], axis=0))
                heads[p] = [ov[:ROWS].astype(BF16), ov[ROWS:2 * ROWS].astype(BF16)]
                otail[rows, pl.ds(2 * p * DH, DH)] = ov[2 * ROWS:2 * ROWS + TAIL]
                otail[rows, pl.ds((2 * p + 1) * DH, DH)] = ov[2 * ROWS + TAIL:]

            def output(p0, p1):
                o = jnp.concatenate([h for p in range(p0, p1) for h in heads[p]], axis=1)
                return _dot(o, wo_rows(2 * p0 * DH, 2 * (p1 - p0) * DH))

            npair = H // 2
            for p in range(0, npair, 2):
                for pp, m in ((p, 0), (p, 1), (p + 1, 0), (p + 1, 1), (p, 2), (p + 1, 2)):
                    project(pp, m)
                scores(p)
                scores(p + 1)
                if p:
                    values(p - 2, pad)
                    values(p - 1, pad)
                else:
                    norm_body(jnp.minimum(s + 1, NSEG - 1))
            a = output(0, npair // 2)
            bits = pltpu.bitcast(a[:pad.shape[0] // 2, 2 * DH:3 * DH], U32)
            late_pad = _packed((bits >> 16) >> 16)
            values(npair - 2, late_pad)
            values(npair - 1, late_pad)
            a = a + output(npair // 2, npair)
            act[s, body, :] = a[M:]
            return a[:M]

        lax.fori_loop(0, NSEG, segment, mem_v[...].astype(F32))

    pl.run_scoped(
        attention,
        pltpu.VMEM((NSTAGE, D, OCT, DH), BF16),
        pltpu.VMEM((3 * NO, D // 2, OCT * DH), U32),
        pltpu.VMEM((NT // 2, D), U32),
        pltpu.VMEM((3 * NO, NT, OCT * DH // 2), U32),
        pltpu.VMEM((2 * (M + SEG), LANES), F32),
        pltpu.SemaphoreType.DMA((NSTAGE,)),
    )

    def mixer(xn, hb, hh, z, ostage, osem):
        def last_modulation(j, carry):
            cp_mod(2 + j, j).wait()
            modulation(2 + j, j)
            return carry

        lax.fori_loop(0, 4, last_modulation, 0)
        for cp in cp_w:
            cp.wait()
        gate_a, shift, gain, gate_b = mod[2][:1], mod[3][:1], 1.0 + mod[4][:1], mod[5][:1]
        hh[0] = jnp.zeros((SEG, D), F32)
        hh[NSEG + 1] = jnp.zeros((SEG, D), F32)

        def token_mlp(i, carry):
            def group(part, a=None):
                ys = []
                for s in range(0, SB, 2):
                    segs = pl.ds(i * SB + s, 2)
                    att = (act[segs, part, :].reshape(2 * TAIL, D) if a is None
                           else a[s * TAIL:(s + 2) * TAIL])
                    x = x_v[segs, part, :].astype(F32).reshape(2 * TAIL, D) + gate_a * att
                    xn[segs, part, :] = x.reshape(2, TAIL, D)
                    h = _layernorm(x) * gain + shift
                    hb[segs, part, :] = h.reshape(2, TAIL, D)
                    ys.append(_layernorm(h).astype(BF16))
                u = _gelu(_dot(jnp.concatenate(ys, axis=0), w1_v[...]))
                hh[pl.ds(1 + i * SB, SB), part, :] = u.reshape(SB, TAIL, D)

            rows = pl.ds(pl.multiple_of(i * SB * TAIL, SB * TAIL), SB * TAIL)
            a_tail = _dot(otail[rows, :].astype(BF16), wo_rows(0, H * DH))
            for t in range(0, BODY, TAIL):
                group(pl.ds(t, TAIL))
            group(tail, a_tail)
            return carry

        lax.fori_loop(0, NSEG // SB, token_mlp, 0)

        def shift_mix(i, carry):
            n = RB2 // SEG
            segs = pl.ds(i * n, n)
            g = D // 4
            shifted = [
                hh[pl.ds(i * n, n + 2), :, pl.ds(j * g, g)].reshape(RB2 + 2 * SEG, g)
                [SEG + d:SEG + d + RB2] for j, d in enumerate((-1, 1, -2, 2))]
            hs = _dot(jnp.concatenate(shifted, axis=1).astype(BF16), w2_v[...])
            hb[segs] = hb[segs] + hs.reshape(n, SEG, D)
            return carry

        lax.fori_loop(0, S // RB2, shift_mix, 0)

        def cp_out(i):
            return pltpu.make_async_copy(
                ostage.at[i % 2], out_hbm.at[pl.ds(pl.multiple_of(i * RB, RB), RB), :],
                osem.at[i % 2])

        def norm_block(i, slot):
            x1 = hb[pl.ds(i * (RB // SEG), RB // SEG)].reshape(RB, D)
            z[slot] = pltpu.bitcast(_layernorm(x1).astype(BF16), U32)

        def channel_mlp(i, carry):
            @pl.when(i >= 2)
            def _():
                cp_out(i - 2).wait()

            segs = pl.ds(i * (RB // SEG), RB // SEG)
            lhs = _packed(z[i % 2])
            y = hb[segs].reshape(RB, D)
            for f in range(F // FC):
                u = _gelu(_dot(lhs, w3_v[:, pl.ds(f * FC, FC)])).astype(BF16)
                y = y + _dot(u, w4_v[pl.ds(f * FC, FC), :])
            norm_block(jnp.minimum(i + 1, S // RB - 1), (i + 1) % 2)
            ostage[i % 2] = (xn[segs].reshape(RB, D) + gate_b * y).astype(BF16)
            cp_out(i).start()
            return carry

        norm_block(0, 0)
        lax.fori_loop(0, S // RB, channel_mlp, 0)
        cp_out(S // RB - 2).wait()
        cp_out(S // RB - 1).wait()

    pl.run_scoped(
        mixer,
        pltpu.VMEM((NSEG, SEG, D), F32),
        pltpu.VMEM((NSEG, SEG, D), F32),
        pltpu.VMEM((NSEG + 2, SEG, D), F32),
        pltpu.VMEM((2, RB // 2, D), U32),
        pltpu.VMEM((2, RB, D), BF16),
        pltpu.SemaphoreType.DMA((2,)),
    )


@jax.jit
def pallas_adaLN_cond__memory_aug_recurrent_mem_tr__mixer_s_mlp__prompt_kernel(
    A_x: jax.Array,
    A_mem0: jax.Array,
    A_Wq: jax.Array,
    A_Wk: jax.Array,
    A_Wv: jax.Array,
    A_Wo: jax.Array,
    A_seg_len: jax.Array,
    B_x: jax.Array,
    B_w1: jax.Array,
    B_w2: jax.Array,
    B_w3: jax.Array,
    B_w4: jax.Array,
    c: jax.Array,
    w_mod: jax.Array,
):
    del A_seg_len, B_x
    B, S, D = A_x.shape
    M = A_mem0.shape[1]
    _, H, DH = A_Wq.shape
    F = B_w3.shape[1]
    assert B == 1 and M == 8 and DH == LANES and S % RB2 == 0 and F % FC == 0

    out = pl.pallas_call(
        _kernel,
        out_shape=jax.ShapeDtypeStruct((S, D), A_x.dtype),
        in_specs=[pl.BlockSpec(memory_space=pl.ANY)] * 12,
        out_specs=pl.BlockSpec(memory_space=pl.ANY),
        scratch_shapes=[
            pltpu.VMEM((S // SEG, SEG, D), BF16),
            pltpu.VMEM((S // SEG, SEG, D), F32),
            pltpu.VMEM((S // SEG * TAIL, H * DH), F32),
            pltpu.VMEM((4, D, D), BF16),
            pltpu.VMEM((D // LANES, H * DH, LANES), BF16),
            pltpu.VMEM((D, D), BF16),
            pltpu.VMEM((D, D), BF16),
            pltpu.VMEM((D, F), BF16),
            pltpu.VMEM((F, D), BF16),
            pltpu.VMEM((1, D), BF16),
            pltpu.VMEM((M, D), BF16),
            pltpu.VMEM((6, 8, D), F32),
            pltpu.SemaphoreType.DMA((12 + D // LANES,)),
        ],
        compiler_params=pltpu.CompilerParams(vmem_limit_bytes=124 * 2**20),
    )(A_x.reshape(S // SEG, SEG, D), A_mem0.reshape(M, D), A_Wq, A_Wk, A_Wv,
      A_Wo.reshape(H * DH, D), B_w1, B_w2, B_w3, B_w4, c, w_mod)
    return out.reshape(B, S, D)
```

```python
import math

import jax
import jax.numpy as jnp
from jax import lax
import jax.experimental.pallas as pl
import jax.experimental.pallas.tpu as pltpu

F32, BF16, U32 = jnp.float32, jnp.bfloat16, jnp.uint32

SEG = 32
TAIL = 8
BODY = SEG - TAIL
OCT = 8
LANES = 128
NSTAGE = 2
SB = 16
RB2 = 512
RB = 128
TG = 4
EPS = 1e-5


def _layernorm(x):
    m = jnp.mean(x, axis=-1, keepdims=True)
    d = x - m
    v = jnp.mean(d * d, axis=-1, keepdims=True)
    return d * lax.rsqrt(v + EPS)


def _gelu(x):
    c1 = math.sqrt(2.0 / math.pi)
    hx = 0.5 * x
    return hx + hx * jnp.tanh(x * (c1 + (c1 * 0.044715) * (x * x)))


def _dot(a, b):
    return jnp.dot(a, b, preferred_element_type=F32)


def _packed(words):
    return pltpu.bitcast(words, BF16)


def _kernel(x_hbm, mem_hbm, wq_hbm, wk_hbm, wv_hbm, wo_hbm, w1_hbm, w2_hbm, w3_hbm, w4_hbm,
            c_hbm, wmod_hbm, out_hbm,
            x_v, act, wqkv, pre, wo_v, w1_v, w2_v, w3_v, w4_v, c_v, mem_v, mod, fill, sem):
    NSEG, _, D = x_hbm.shape
    _, H, DH = wq_hbm.shape
    M = mem_hbm.shape[0]
    S = NSEG * SEG
    F = w3_hbm.shape[1]
    NO = H // OCT
    ROWS = M + BODY
    NT = NSEG * TAIL
    scale = DH ** -0.5
    body, tail = pl.ds(0, BODY), pl.ds(BODY, TAIL)

    def copy(src, dst, i):
        return pltpu.make_async_copy(src, dst, sem.at[i])

    cp_c = copy(c_hbm, c_v, 0)
    cp_mem = copy(mem_hbm, mem_v, 1)
    cp_xt = copy(x_hbm.at[:, tail, :], x_v.at[:, tail, :], 2)
    cp_xb = copy(x_hbm.at[:, body, :], x_v.at[:, body, :], 3)
    cp_w = [copy(w1_hbm, w1_v, 4), copy(w2_hbm, w2_v, 5), copy(w3_hbm, w3_v, 6),
            copy(w4_hbm, w4_v, 7)]

    def cp_wo(n):
        return copy(wo_hbm.at[:, pl.ds(pl.multiple_of(n * LANES, LANES), LANES)], wo_v.at[n], 8 + n)

    def wo_rows(r0, n):
        return jnp.concatenate([wo_v[j, pl.ds(r0, n), :] for j in range(D // LANES)], axis=1)

    def prologue(stage, wmod_v, ht, wsem, msem):
        def cp_mod(j):
            return pltpu.make_async_copy(
                wmod_hbm.at[:, pl.ds(pl.multiple_of(j * D, D), D)], wmod_v.at[j % 4],
                msem.at[j % 4])

        def modulation(j, carry):
            cp_mod(j).wait()

            @pl.when(j == 0)
            def _():
                cp_oct(wq_hbm, 1, 1).start()

            c = c_v[...].astype(F32)
            sc = jnp.broadcast_to(c * jax.nn.sigmoid(c), (16, D)).astype(BF16)
            mod[j] = _dot(sc, wmod_v[j % 4])[:8]
            return carry

        def cp_oct(w_hbm, o, slot):
            return pltpu.make_async_copy(
                w_hbm.at[:, pl.ds(pl.multiple_of(o * OCT, OCT), OCT), :], stage.at[slot],
                wsem.at[slot])

        def relayout(i, b, n):
            w = stage[i % NSTAGE, pl.ds(pl.multiple_of(b * n, n), n), :, :].reshape(n * OCT, DH)
            w = jnp.swapaxes(pltpu.bitcast(w, U32).reshape(n // 2, OCT, DH), 0, 1)
            rows = pl.ds(pl.multiple_of(b * (n // 2), n // 2), n // 2)
            for j in range(OCT // 2):
                even, odd = w[j], w[OCT // 2 + j]
                wqkv[i, rows, pl.ds(2 * j * DH, DH)] = (even & 0xFFFF) | (odd << 16)
                wqkv[i, rows, pl.ds((2 * j + 1) * DH, DH)] = (even >> 16) | ((odd >> 16) << 16)

        cp_oct(wq_hbm, 0, 0).start()
        cp_xt.start()
        cp_c.start()
        cp_mem.start()

        def head_pos(i):
            head = jnp.where(i < 2 * ROWS, i // ROWS, (i - 2 * ROWS) // TAIL)
            pos = jnp.where(i < 2 * ROWS, i % ROWS, ROWS + i % TAIL)
            return head, pos

        hr, pr = head_pos(lax.broadcasted_iota(jnp.int32, fill.shape, 0))
        hc, pc = head_pos(lax.broadcasted_iota(jnp.int32, fill.shape, 1))
        visible = (pr < M) | (pr >= pc)
        fill[...] = jnp.where(hr == hc, jnp.where(visible, 0.0, -1e9 / scale), -jnp.inf)

        def first_relayout(b, carry):
            relayout(0, b, D // OCT)
            return carry

        def norm_tail(i, carry):
            segs = pl.ds(i * 8, 8)
            xt = x_v[segs, tail, :].astype(F32).reshape(8 * TAIL, D)
            act[segs, tail, :] = _layernorm(xt).reshape(8, TAIL, D)
            return carry

        cp_xt.wait()
        cp_mod(0).start()
        lax.fori_loop(0, NSEG // 8, norm_tail, 0)
        cp_oct(wq_hbm, 0, 0).wait()
        cp_mod(1).start()
        lax.fori_loop(0, OCT, first_relayout, 0)
        cp_c.wait()
        lax.fori_loop(0, 2, modulation, 0)
        shift, gain = mod[0][:1], 1.0 + mod[1][:1]
        ht[...] = pltpu.bitcast((act[:, tail, :].reshape(NT, D) * gain + shift).astype(BF16), U32)

        def project_tail(i, carry):
            @pl.when(i + 1 < 3 * NO)
            def _():
                cp_oct(wq_hbm, 0, (i + 1) % NSTAGE).wait()

            for m, w_hbm in enumerate((wq_hbm, wk_hbm, wv_hbm)):
                @pl.when((i + 2) // NO == m)
                def _():
                    cp_oct(w_hbm, (i + 2) % NO, (i + 2) % NSTAGE).start()

            @pl.when(i < D // LANES)
            def _():
                cp_wo(i).start()

            @pl.when(i == D // LANES)
            def _():
                cp_xb.start()

            @pl.when(i == 3 * NO - 3)
            def _():
                for j in range(2, 6):
                    cp_mod(j).start()

            nxt = jnp.minimum(i + 1, 3 * NO - 1)
            n = NT // TG
            for j in range(OCT // 2):
                for g in range(TG):
                    lhs = _packed(ht[pl.ds(g * n // 2, n // 2), :])
                    halves = []
                    for h in (2 * j, 2 * j + 1):
                        r = _dot(lhs, _packed(wqkv[i, :, pl.ds(h * DH, DH)]))
                        halves.append(r.reshape(n // TAIL, TAIL, DH))
                        relayout(nxt, h * TG + g, D // (OCT * TG))
                    r = jnp.concatenate(halves, axis=1).reshape(2 * n, DH).astype(BF16)
                    pre[i, pl.ds(g * n, n), pl.ds(j * DH, DH)] = pltpu.bitcast(r, U32)
            return carry

        lax.fori_loop(0, 3 * NO, project_tail, 0)

        lax.fori_loop(2, 6, modulation, 0)

    pl.run_scoped(
        prologue,
        pltpu.VMEM((NSTAGE, D, OCT, DH), BF16),
        pltpu.VMEM((4, D, D), BF16),
        pltpu.VMEM((NT // 2, D), U32),
        pltpu.SemaphoreType.DMA((NSTAGE,)),
        pltpu.SemaphoreType.DMA((4,)),
    )

    def main(otail, xn, hb, yb, hh, mean, ostage, osem):
        def norm_body(s):
            act[s, body, :] = (_layernorm(x_v[s, body, :].astype(F32)) * (1.0 + mod[1][:1])
                               + mod[0][:1])

        def mixer_input(x, att):
            x = x.astype(F32) + mod[2][:1] * att
            h = _layernorm(x) * (1.0 + mod[4][:1]) + mod[3][:1]
            return x, h, _layernorm(h)

        def mixer_input_body(s):
            xn[s, body, :], hb[s, body, :], yb[s] = mixer_input(x_v[s, body, :], act[s, body, :])

        cp_xb.wait()
        cp_mem.wait()
        for n in range(D // LANES):
            cp_wo(n).wait()
        for cp in cp_w:
            cp.start()
        norm_body(0)

        def segment(s, mem):
            lhs = jnp.concatenate([mem, act[s, body, :]], axis=0).astype(BF16)
            rows = pl.ds(pl.multiple_of(s * TAIL, TAIL), TAIL)
            pad = jnp.zeros((fill.shape[1] - fill.shape[0], DH), BF16)
            qkv, probs, heads = {}, {}, {}

            def project(p, m):
                o, j = divmod(p, OCT // 2)
                r = _dot(lhs, _packed(wqkv[m * NO + o, :, pl.ds(2 * j * DH, 2 * DH)]))
                r = r.astype(BF16)
                t = _packed(pre[m * NO + o, rows, pl.ds(j * DH, DH)])
                qkv[p, m] = [r[:, :DH], r[:, DH:], t]

            def scores(p):
                q = jnp.concatenate(qkv[p, 0], axis=0)
                k = jnp.concatenate(qkv[p, 1] + [pad], axis=0)
                sc = lax.dot_general(q, k, (((1,), (1,)), ((), ())), preferred_element_type=F32)
                f = fill[...]
                sc = jnp.where(f == 0.0, sc, f)
                e = jnp.exp2((sc - jnp.max(sc, axis=-1, keepdims=True))
                             * (scale * math.log2(math.e)))
                inv = pltpu.reciprocal(jnp.sum(e, axis=-1, keepdims=True), full_range=False)
                probs[p] = (e * inv).astype(BF16)

            def values(p, pad):
                ov = _dot(probs[p], jnp.concatenate(qkv[p, 2] + [pad], axis=0))
                heads[p] = [ov[:ROWS].astype(BF16), ov[ROWS:2 * ROWS].astype(BF16)]
                otail[rows, pl.ds(2 * p * DH, DH)] = ov[2 * ROWS:2 * ROWS + TAIL]
                otail[rows, pl.ds((2 * p + 1) * DH, DH)] = ov[2 * ROWS + TAIL:]

            def output(p0, p1):
                o = jnp.concatenate([h for p in range(p0, p1) for h in heads[p]], axis=1)
                return _dot(o, wo_rows(2 * p0 * DH, 2 * (p1 - p0) * DH))

            npair = H // 2
            for p in range(0, npair, 2):
                for pp, m in ((p, 0), (p, 1), (p + 1, 0), (p + 1, 1), (p, 2), (p + 1, 2)):
                    project(pp, m)
                scores(p)
                scores(p + 1)
                if p:
                    values(p - 2, pad)
                    values(p - 1, pad)
                else:
                    mixer_input_body(jnp.maximum(s - 1, 0))
                    norm_body(jnp.minimum(s + 1, NSEG - 1))
            a = output(0, npair // 2)
            bits = pltpu.bitcast(a[:pad.shape[0] // 2, 2 * DH:3 * DH], U32)
            late_pad = _packed((bits >> 16) >> 16)
            values(npair - 2, late_pad)
            values(npair - 1, late_pad)
            a = a + output(npair // 2, npair)
            act[s, body, :] = a[M:]
            return a[:M]

        lax.fori_loop(0, NSEG, segment, mem_v[...].astype(F32))

        mixer_input_body(NSEG - 1)
        for cp in cp_w:
            cp.wait()
        hh[0] = jnp.zeros((SEG, D), F32)
        hh[NSEG + 1] = jnp.zeros((SEG, D), F32)

        def token_mlp(i, carry):
            segs, out = pl.ds(i * SB, SB), pl.ds(1 + i * SB, SB)
            rows = pl.ds(pl.multiple_of(i * SB * TAIL, SB * TAIL), SB * TAIL)
            att = _dot(otail[rows, :].astype(BF16), wo_rows(0, H * DH))
            y = yb[segs].reshape(SB * BODY, D).astype(BF16)
            hh[out, body, :] = _gelu(_dot(y, w1_v[...])).reshape(SB, BODY, D)
            x, h, y = mixer_input(x_v[segs, tail, :].reshape(SB * TAIL, D), att)
            xn[segs, tail, :] = x.reshape(SB, TAIL, D)
            hb[segs, tail, :] = h.reshape(SB, TAIL, D)
            hh[out, tail, :] = _gelu(_dot(y.astype(BF16), w1_v[...])).reshape(SB, TAIL, D)
            return carry

        lax.fori_loop(0, NSEG // SB, token_mlp, 0)

        def shift_mix(i, carry):
            n = RB2 // SEG
            segs = pl.ds(i * n, n)
            g = D // 4
            shifted = [
                hh[pl.ds(i * n, n + 2), :, pl.ds(j * g, g)].reshape(RB2 + 2 * SEG, g)
                [SEG + d:SEG + d + RB2] for j, d in enumerate((-1, 1, -2, 2))]
            hs = _dot(jnp.concatenate(shifted, axis=1).astype(BF16), w2_v[...])
            x1 = hb[segs].reshape(RB2, D) + hs
            hb[segs] = x1.reshape(n, SEG, D)
            mean[pl.ds(pl.multiple_of(i * RB2, RB2), RB2), :] = jnp.broadcast_to(
                jnp.mean(x1, axis=-1, keepdims=True), (RB2, LANES))
            return carry

        lax.fori_loop(0, S // RB2, shift_mix, 0)

        def cp_out(i):
            return pltpu.make_async_copy(
                ostage.at[i % 2], out_hbm.at[pl.ds(pl.multiple_of(i * RB, RB), RB), :],
                osem.at[i % 2])

        def channel_mlp(i, carry):
            @pl.when(i >= 2)
            def _():
                cp_out(i - 2).wait()

            segs = pl.ds(i * (RB // SEG), RB // SEG)
            x1 = hb[segs].reshape(RB, D)
            m = mean[pl.ds(pl.multiple_of(i * RB, RB), RB), :]
            d = x1 - jnp.concatenate([m] * (D // LANES), axis=1)
            r = lax.rsqrt(jnp.mean(d * d, axis=-1, keepdims=True) + EPS)
            u = _gelu(_dot(d.astype(BF16), w3_v[...]) * r).astype(BF16)
            y = x1 + _dot(u, w4_v[...])
            ostage[i % 2] = (xn[segs].reshape(RB, D) + mod[5][:1] * y).astype(BF16)
            cp_out(i).start()
            return carry

        lax.fori_loop(0, S // RB, channel_mlp, 0)
        cp_out(S // RB - 2).wait()
        cp_out(S // RB - 1).wait()

    pl.run_scoped(
        main,
        pltpu.VMEM((NT, H * DH), F32),
        pltpu.VMEM((NSEG, SEG, D), F32),
        pltpu.VMEM((NSEG, SEG, D), F32),
        pltpu.VMEM((NSEG, BODY, D), F32),
        pltpu.VMEM((NSEG + 2, SEG, D), F32),
        pltpu.VMEM((S, LANES), F32),
        pltpu.VMEM((2, RB, D), BF16),
        pltpu.SemaphoreType.DMA((2,)),
    )


@jax.jit
def pallas_adaLN_cond__memory_aug_recurrent_mem_tr__mixer_s_mlp__prompt_kernel(
    A_x: jax.Array,
    A_mem0: jax.Array,
    A_Wq: jax.Array,
    A_Wk: jax.Array,
    A_Wv: jax.Array,
    A_Wo: jax.Array,
    A_seg_len: jax.Array,
    B_x: jax.Array,
    B_w1: jax.Array,
    B_w2: jax.Array,
    B_w3: jax.Array,
    B_w4: jax.Array,
    c: jax.Array,
    w_mod: jax.Array,
):
    del A_seg_len, B_x
    B, S, D = A_x.shape
    M = A_mem0.shape[1]
    _, H, DH = A_Wq.shape
    F = B_w3.shape[1]
    assert B == 1 and M == 8 and DH == LANES and S % RB2 == 0

    out = pl.pallas_call(
        _kernel,
        out_shape=jax.ShapeDtypeStruct((S, D), A_x.dtype),
        in_specs=[pl.BlockSpec(memory_space=pl.ANY)] * 12,
        out_specs=pl.BlockSpec(memory_space=pl.ANY),
        scratch_shapes=[
            pltpu.VMEM((S // SEG, SEG, D), BF16),
            pltpu.VMEM((S // SEG, SEG, D), F32),
            pltpu.VMEM((3 * H // OCT, D // 2, OCT * DH), U32),
            pltpu.VMEM((3 * H // OCT, S // SEG * TAIL, OCT * DH // 2), U32),
            pltpu.VMEM((D // LANES, H * DH, LANES), BF16),
            pltpu.VMEM((D, D), BF16),
            pltpu.VMEM((D, D), BF16),
            pltpu.VMEM((D, F), BF16),
            pltpu.VMEM((F, D), BF16),
            pltpu.VMEM((1, D), BF16),
            pltpu.VMEM((M, D), BF16),
            pltpu.VMEM((6, 8, D), F32),
            pltpu.VMEM((2 * (M + SEG), LANES), F32),
            pltpu.SemaphoreType.DMA((8 + D // LANES,)),
        ],
        compiler_params=pltpu.CompilerParams(vmem_limit_bytes=127 * 2**20),
    )(A_x.reshape(S // SEG, SEG, D), A_mem0.reshape(M, D), A_Wq, A_Wk, A_Wv,
      A_Wo.reshape(H * DH, D), B_w1, B_w2, B_w3, B_w4, c, w_mod)
    return out.reshape(B, S, D)
```

```python
import math

import jax
import jax.numpy as jnp
from jax import lax
import jax.experimental.pallas as pl
import jax.experimental.pallas.tpu as pltpu

F32, BF16, U32 = jnp.float32, jnp.bfloat16, jnp.uint32

SEG = 32
TAIL = 8
BODY = SEG - TAIL
OCT = 8
LANES = 128
NSTAGE = 4
SB = 16
RB2 = 512
RB = 128
TG = 4
EPS = 1e-5


def _layernorm(x):
    m = jnp.mean(x, axis=-1, keepdims=True)
    d = x - m
    v = jnp.mean(d * d, axis=-1, keepdims=True)
    return d * lax.rsqrt(v + EPS)


def _gelu(x):
    c1 = math.sqrt(2.0 / math.pi)
    hx = 0.5 * x
    return hx + hx * jnp.tanh(x * (c1 + (c1 * 0.044715) * (x * x)))


def _dot(a, b):
    return jnp.dot(a, b, preferred_element_type=F32)


def _packed(words):
    return pltpu.bitcast(words, BF16)


def _kernel(x_hbm, mem_hbm, wq_hbm, wk_hbm, wv_hbm, wo_hbm, w1_hbm, w2_hbm, w3_hbm, w4_hbm,
            c_hbm, wmod_hbm, out_hbm,
            x_v, act, wqkv, pre, wo_v, w1_v, w2_v, w3_v, w4_v, c_v, mem_v, mod, fill, sem):
    NSEG, _, D = x_hbm.shape
    _, H, DH = wq_hbm.shape
    M = mem_hbm.shape[0]
    S = NSEG * SEG
    F = w3_hbm.shape[1]
    NO = H // OCT
    ROWS = M + BODY
    NT = NSEG * TAIL
    scale = DH ** -0.5
    body, tail = pl.ds(0, BODY), pl.ds(BODY, TAIL)

    def copy(src, dst, i):
        return pltpu.make_async_copy(src, dst, sem.at[i])

    cp_c = copy(c_hbm, c_v, 0)
    cp_mem = copy(mem_hbm, mem_v, 1)
    cp_xt = copy(x_hbm.at[:, tail, :], x_v.at[:, tail, :], 2)
    cp_w = [copy(w1_hbm, w1_v, 4), copy(w2_hbm, w2_v, 5), copy(w3_hbm, w3_v, 6),
            copy(w4_hbm, w4_v, 7)]

    def cp_wo(n):
        return copy(wo_hbm.at[:, pl.ds(pl.multiple_of(n * LANES, LANES), LANES)], wo_v.at[n], 8 + n)

    def cp_xb(n):
        segs = pl.ds(n * (NSEG * LANES // D), NSEG * LANES // D)
        return copy(x_hbm.at[segs, body, :], x_v.at[segs, body, :], 8 + D // LANES + n)

    def wo_rows(r0, n):
        return jnp.concatenate([wo_v[j, pl.ds(r0, n), :] for j in range(D // LANES)], axis=1)

    def prologue(stage, wmod_v, ht, wsem, msem):
        def cp_mod(j):
            return pltpu.make_async_copy(
                wmod_hbm.at[:, pl.ds(pl.multiple_of(j * D, D), D)], wmod_v.at[j % 4],
                msem.at[j % 4])

        def modulation(j, carry):
            cp_mod(j).wait()

            @pl.when(j == 1)
            def _():
                cp_oct(wq_hbm, 1, 1).start()

            c = c_v[...].astype(F32)
            sc = jnp.broadcast_to(c * jax.nn.sigmoid(c), (16, D)).astype(BF16)
            mod[j] = _dot(sc, wmod_v[j % 4])[:8]
            return carry

        def cp_oct(w_hbm, o, slot):
            return pltpu.make_async_copy(
                w_hbm.at[:, pl.ds(pl.multiple_of(o * OCT, OCT), OCT), :], stage.at[slot],
                wsem.at[slot])

        def relayout(i, b, n):
            w = stage[i % NSTAGE, pl.ds(pl.multiple_of(b * n, n), n), :, :].reshape(n * OCT, DH)
            w = jnp.swapaxes(pltpu.bitcast(w, U32).reshape(n // 2, OCT, DH), 0, 1)
            rows = pl.ds(pl.multiple_of(b * (n // 2), n // 2), n // 2)
            for j in range(OCT // 2):
                even, odd = w[j], w[OCT // 2 + j]
                wqkv[i, rows, pl.ds(2 * j * DH, DH)] = (even & 0xFFFF) | (odd << 16)
                wqkv[i, rows, pl.ds((2 * j + 1) * DH, DH)] = (even >> 16) | ((odd >> 16) << 16)

        cp_oct(wq_hbm, 0, 0).start()
        cp_xt.start()
        cp_c.start()
        cp_mem.start()

        def head_pos(i):
            head = jnp.where(i < 2 * ROWS, i // ROWS, (i - 2 * ROWS) // TAIL)
            pos = jnp.where(i < 2 * ROWS, i % ROWS, ROWS + i % TAIL)
            return head, pos

        hr, pr = head_pos(lax.broadcasted_iota(jnp.int32, fill.shape, 0))
        hc, pc = head_pos(lax.broadcasted_iota(jnp.int32, fill.shape, 1))
        visible = (pr < M) | (pr >= pc)
        fill[...] = jnp.where(hr == hc, jnp.where(visible, 0.0, -1e9 / scale), -jnp.inf)

        def whole_relayout(b, i):
            relayout(i, b, D // OCT)
            return i

        def norm_tail(i, carry):
            segs = pl.ds(i * 8, 8)
            xt = x_v[segs, tail, :].astype(F32).reshape(8 * TAIL, D)
            act[segs, tail, :] = _layernorm(xt).reshape(8, TAIL, D)
            return carry

        cp_xt.wait()
        cp_mod(0).start()
        lax.fori_loop(0, NSEG // 8, norm_tail, 0)
        cp_oct(wq_hbm, 0, 0).wait()
        cp_mod(1).start()
        lax.fori_loop(0, OCT, whole_relayout, 0)
        cp_c.wait()
        lax.fori_loop(0, 2, modulation, 0)
        shift, gain = mod[0][:1], 1.0 + mod[1][:1]
        ht[...] = pltpu.bitcast((act[:, tail, :].reshape(NT, D) * gain + shift).astype(BF16), U32)

        def project_tail(i, carry):
            @pl.when(i == 1)
            def _():
                cp_oct(wq_hbm, 1, 1).wait()
                lax.fori_loop(0, OCT, whole_relayout, 1)

            @pl.when((i > 0) & (i + 1 < 3 * NO))
            def _():
                cp_oct(wq_hbm, 0, (i + 1) % NSTAGE).wait()

            for m, w_hbm in enumerate((wq_hbm, wk_hbm, wv_hbm)):
                @pl.when((i + 2) // NO == m)
                def _():
                    cp_oct(w_hbm, (i + 2) % NO, (i + 2) % NSTAGE).start()

            @pl.when((i > 0) & (i <= D // LANES))
            def _():
                cp_wo(i - 1).start()
                cp_xb(i - 1).start()

            @pl.when((i > D // LANES) & (i <= D // LANES + 2))
            def _():
                cp_mod(2 * (i - D // LANES)).start()
                cp_mod(2 * (i - D // LANES) + 1).start()

            nxt = jnp.where(i == 0, 0, jnp.minimum(i + 1, 3 * NO - 1))
            n = NT // TG
            for j in range(OCT // 2):
                for g in range(TG):
                    lhs = _packed(ht[pl.ds(g * n // 2, n // 2), :])
                    halves = []
                    for h in (2 * j, 2 * j + 1):
                        r = _dot(lhs, _packed(wqkv[i, :, pl.ds(h * DH, DH)]))
                        halves.append(r.reshape(n // TAIL, TAIL, DH))
                        relayout(nxt, h * TG + g, D // (OCT * TG))
                    r = jnp.concatenate(halves, axis=1).reshape(2 * n, DH).astype(BF16)
                    pre[i, pl.ds(g * n, n), pl.ds(j * DH, DH)] = pltpu.bitcast(r, U32)
            return carry

        lax.fori_loop(0, 3 * NO, project_tail, 0)

        lax.fori_loop(2, 6, modulation, 0)

    pl.run_scoped(
        prologue,
        pltpu.VMEM((NSTAGE, D, OCT, DH), BF16),
        pltpu.VMEM((4, D, D), BF16),
        pltpu.VMEM((NT // 2, D), U32),
        pltpu.SemaphoreType.DMA((NSTAGE,)),
        pltpu.SemaphoreType.DMA((4,)),
    )

    def main(otail, xn, hb, yb, hh, mean, ostage, osem):
        def norm_body(s):
            act[s, body, :] = (_layernorm(x_v[s, body, :].astype(F32)) * (1.0 + mod[1][:1])
                               + mod[0][:1])

        def mixer_input(x, att):
            x = x.astype(F32) + mod[2][:1] * att
            h = _layernorm(x) * (1.0 + mod[4][:1]) + mod[3][:1]
            return x, h, _layernorm(h)

        def mixer_input_body(s):
            xn[s, body, :], hb[s, body, :], yb[s] = mixer_input(x_v[s, body, :], act[s, body, :])

        cp_mem.wait()
        for n in range(D // LANES):
            cp_wo(n).wait()
            cp_xb(n).wait()
        for cp in cp_w:
            cp.start()
        norm_body(0)

        def segment(s, mem):
            lhs = jnp.concatenate([mem, act[s, body, :]], axis=0).astype(BF16)
            rows = pl.ds(pl.multiple_of(s * TAIL, TAIL), TAIL)
            pad = jnp.zeros((fill.shape[1] - fill.shape[0], DH), BF16)
            qkv, probs, heads = {}, {}, {}

            def project(p, m):
                o, j = divmod(p, OCT // 2)
                r = _dot(lhs, _packed(wqkv[m * NO + o, :, pl.ds(2 * j * DH, 2 * DH)]))
                r = r.astype(BF16)
                t = _packed(pre[m * NO + o, rows, pl.ds(j * DH, DH)])
                qkv[p, m] = [r[:, :DH], r[:, DH:], t]

            def scores(p):
                q = jnp.concatenate(qkv[p, 0], axis=0)
                k = jnp.concatenate(qkv[p, 1] + [pad], axis=0)
                sc = lax.dot_general(q, k, (((1,), (1,)), ((), ())), preferred_element_type=F32)
                f = fill[...]
                sc = jnp.where(f == 0.0, sc, f)
                e = jnp.exp2((sc - jnp.max(sc, axis=-1, keepdims=True))
                             * (scale * math.log2(math.e)))
                inv = pltpu.reciprocal(jnp.sum(e, axis=-1, keepdims=True), full_range=False)
                probs[p] = (e * inv).astype(BF16)

            def values(p, pad):
                ov = _dot(probs[p], jnp.concatenate(qkv[p, 2] + [pad], axis=0))
                heads[p] = [ov[:ROWS].astype(BF16), ov[ROWS:2 * ROWS].astype(BF16)]
                otail[rows, pl.ds(2 * p * DH, DH)] = ov[2 * ROWS:2 * ROWS + TAIL]
                otail[rows, pl.ds((2 * p + 1) * DH, DH)] = ov[2 * ROWS + TAIL:]

            def output(p0, p1):
                o = jnp.concatenate([h for p in range(p0, p1) for h in heads[p]], axis=1)
                return _dot(o, wo_rows(2 * p0 * DH, 2 * (p1 - p0) * DH))

            npair = H // 2
            for p in range(0, npair, 2):
                for pp, m in ((p, 0), (p, 1), (p + 1, 0), (p + 1, 1), (p, 2), (p + 1, 2)):
                    project(pp, m)
                scores(p)
                scores(p + 1)
                if p:
                    values(p - 2, pad)
                    values(p - 1, pad)
                else:
                    mixer_input_body(jnp.maximum(s - 1, 0))
                    norm_body(jnp.minimum(s + 1, NSEG - 1))
            a = output(0, npair // 2)
            bits = pltpu.bitcast(a[:pad.shape[0] // 2, 2 * DH:3 * DH], U32)
            late_pad = _packed((bits >> 16) >> 16)
            values(npair - 2, late_pad)
            values(npair - 1, late_pad)
            a = a + output(npair // 2, npair)
            act[s, body, :] = a[M:]
            return a[:M]

        lax.fori_loop(0, NSEG, segment, mem_v[...].astype(F32))

        mixer_input_body(NSEG - 1)
        for cp in cp_w:
            cp.wait()
        hh[0] = jnp.zeros((SEG, D), F32)
        hh[NSEG + 1] = jnp.zeros((SEG, D), F32)

        def token_mlp(i, carry):
            segs, out = pl.ds(i * SB, SB), pl.ds(1 + i * SB, SB)
            rows = pl.ds(pl.multiple_of(i * SB * TAIL, SB * TAIL), SB * TAIL)
            att = _dot(otail[rows, :].astype(BF16), wo_rows(0, H * DH))
            y = yb[segs].reshape(SB * BODY, D).astype(BF16)
            hh[out, body, :] = _gelu(_dot(y, w1_v[...])).reshape(SB, BODY, D)
            x, h, y = mixer_input(x_v[segs, tail, :].reshape(SB * TAIL, D), att)
            xn[segs, tail, :] = x.reshape(SB, TAIL, D)
            hb[segs, tail, :] = h.reshape(SB, TAIL, D)
            hh[out, tail, :] = _gelu(_dot(y.astype(BF16), w1_v[...])).reshape(SB, TAIL, D)
            return carry

        lax.fori_loop(0, NSEG // SB, token_mlp, 0)

        def shift_mix(i, carry):
            n = RB2 // SEG
            segs = pl.ds(i * n, n)
            g = D // 4
            shifted = [
                hh[pl.ds(i * n, n + 2), :, pl.ds(j * g, g)].reshape(RB2 + 2 * SEG, g)
                [SEG + d:SEG + d + RB2] for j, d in enumerate((-1, 1, -2, 2))]
            hs = _dot(jnp.concatenate(shifted, axis=1).astype(BF16), w2_v[...])
            x1 = hb[segs].reshape(RB2, D) + hs
            hb[segs] = x1.reshape(n, SEG, D)
            mean[pl.ds(pl.multiple_of(i * RB2, RB2), RB2), :] = jnp.broadcast_to(
                jnp.mean(x1, axis=-1, keepdims=True), (RB2, LANES))
            return carry

        lax.fori_loop(0, S // RB2, shift_mix, 0)

        def cp_out(i):
            return pltpu.make_async_copy(
                ostage.at[i % 2], out_hbm.at[pl.ds(pl.multiple_of(i * RB, RB), RB), :],
                osem.at[i % 2])

        def channel_mlp(i, carry):
            @pl.when(i >= 2)
            def _():
                cp_out(i - 2).wait()

            segs = pl.ds(i * (RB // SEG), RB // SEG)
            x1 = hb[segs].reshape(RB, D)
            m = mean[pl.ds(pl.multiple_of(i * RB, RB), RB), :]
            d = x1 - jnp.concatenate([m] * (D // LANES), axis=1)
            r = lax.rsqrt(jnp.mean(d * d, axis=-1, keepdims=True) + EPS)
            u = _gelu(_dot(d.astype(BF16), w3_v[...]) * r).astype(BF16)
            y = x1 + _dot(u, w4_v[...])
            ostage[i % 2] = (xn[segs].reshape(RB, D) + mod[5][:1] * y).astype(BF16)
            cp_out(i).start()
            return carry

        lax.fori_loop(0, S // RB, channel_mlp, 0)
        cp_out(S // RB - 2).wait()
        cp_out(S // RB - 1).wait()

    pl.run_scoped(
        main,
        pltpu.VMEM((NT, H * DH), F32),
        pltpu.VMEM((NSEG, SEG, D), F32),
        pltpu.VMEM((NSEG, SEG, D), F32),
        pltpu.VMEM((NSEG, BODY, D), F32),
        pltpu.VMEM((NSEG + 2, SEG, D), F32),
        pltpu.VMEM((S, LANES), F32),
        pltpu.VMEM((2, RB, D), BF16),
        pltpu.SemaphoreType.DMA((2,)),
    )


@jax.jit
def pallas_adaLN_cond__memory_aug_recurrent_mem_tr__mixer_s_mlp__prompt_kernel(
    A_x: jax.Array,
    A_mem0: jax.Array,
    A_Wq: jax.Array,
    A_Wk: jax.Array,
    A_Wv: jax.Array,
    A_Wo: jax.Array,
    A_seg_len: jax.Array,
    B_x: jax.Array,
    B_w1: jax.Array,
    B_w2: jax.Array,
    B_w3: jax.Array,
    B_w4: jax.Array,
    c: jax.Array,
    w_mod: jax.Array,
):
    del A_seg_len, B_x
    B, S, D = A_x.shape
    M = A_mem0.shape[1]
    _, H, DH = A_Wq.shape
    F = B_w3.shape[1]
    assert B == 1 and M == 8 and DH == LANES and S % RB2 == 0

    out = pl.pallas_call(
        _kernel,
        out_shape=jax.ShapeDtypeStruct((S, D), A_x.dtype),
        in_specs=[pl.BlockSpec(memory_space=pl.ANY)] * 12,
        out_specs=pl.BlockSpec(memory_space=pl.ANY),
        scratch_shapes=[
            pltpu.VMEM((S // SEG, SEG, D), BF16),
            pltpu.VMEM((S // SEG, SEG, D), F32),
            pltpu.VMEM((3 * H // OCT, D // 2, OCT * DH), U32),
            pltpu.VMEM((3 * H // OCT, S // SEG * TAIL, OCT * DH // 2), U32),
            pltpu.VMEM((D // LANES, H * DH, LANES), BF16),
            pltpu.VMEM((D, D), BF16),
            pltpu.VMEM((D, D), BF16),
            pltpu.VMEM((D, F), BF16),
            pltpu.VMEM((F, D), BF16),
            pltpu.VMEM((1, D), BF16),
            pltpu.VMEM((M, D), BF16),
            pltpu.VMEM((6, 8, D), F32),
            pltpu.VMEM((2 * (M + SEG), LANES), F32),
            pltpu.SemaphoreType.DMA((8 + 2 * D // LANES,)),
        ],
        compiler_params=pltpu.CompilerParams(vmem_limit_bytes=127 * 2**20),
    )(A_x.reshape(S // SEG, SEG, D), A_mem0.reshape(M, D), A_Wq, A_Wk, A_Wv,
      A_Wo.reshape(H * DH, D), B_w1, B_w2, B_w3, B_w4, c, w_mod)
    return out.reshape(B, S, D)
```

```python
import math

import jax
import jax.numpy as jnp
from jax import lax
import jax.experimental.pallas as pl
import jax.experimental.pallas.tpu as pltpu

F32, BF16, U32 = jnp.float32, jnp.bfloat16, jnp.uint32

SEG = 32
TAIL = 8
BODY = SEG - TAIL
OCT = 8
LANES = 128
NSTAGE = 4
SB = 16
RB2 = 512
RB = 128
TG = 4
EPS = 1e-5
EARLY = 6
C3 = 128
C4 = 256


def _layernorm(x):
    m = jnp.mean(x, axis=-1, keepdims=True)
    d = x - m
    v = jnp.mean(d * d, axis=-1, keepdims=True)
    return d * lax.rsqrt(v + EPS)


def _gelu(x):
    c1 = math.sqrt(2.0 / math.pi)
    hx = 0.5 * x
    return hx + hx * jnp.tanh(x * (c1 + (c1 * 0.044715) * (x * x)))


def _dot(a, b):
    return jnp.dot(a, b, preferred_element_type=F32)


def _packed(words):
    return pltpu.bitcast(words, BF16)


def _strassen_lhs(a11, a12, a21, a22):
    return [a.astype(BF16) for a in
            (a11 + a22, a21 + a22, a11, a22, a11 + a12, a21 - a11, a12 - a22)]


def _strassen_rhs(b11, b12, b21, b22):
    return [b.astype(BF16) for b in (b11 + b22, b12 - b22, b21 - b11, b11 + b12, b21 + b22)]


def _zero_after(words):
    return (words >> 16) >> 16


def _combine_weights(w_ref, s_ref, r0, c0):
    half = w_ref.shape[2] // 2
    quads = [w_ref[t, pl.ds(pl.multiple_of(r0, 16), 16),
                   pl.ds(pl.multiple_of(c + c0, LANES), LANES)].astype(F32)
             for t in range(2) for c in (0, half)]
    parts = [pltpu.bitcast(part, U32) for part in _strassen_rhs(*quads)]
    for n, part in enumerate(parts):
        s_ref[n, pl.ds(pl.multiple_of(r0 // 2, 8), 8),
              pl.ds(pl.multiple_of(c0, LANES), LANES)] = part
    return _zero_after(parts[0] | parts[1] | parts[2] | parts[3] | parts[4])


def _rhs(w_ref, s_ref, n, c0, nc):
    if n == 1:
        return w_ref[0, :, pl.ds(c0, nc)]
    if n == 4:
        return w_ref[1, :, pl.ds(w_ref.shape[2] // 2 + c0, nc)]
    return _packed(s_ref[n - (n > 1) - (n > 4), :, pl.ds(c0, nc)])


def _strassen_out(product):
    p2, p4 = product(1), product(3)
    c21 = p2 + p4
    p1 = product(0)
    c11, c22 = p1 + p4, p1 - p2
    p3 = product(2)
    c22 = c22 + p3
    p5 = product(4)
    c12 = p3 + p5
    c11 = c11 - p5
    c22 = c22 + product(5)
    c11 = c11 + product(6)
    return c11, c12, c21, c22


def _kernel(x_hbm, mem_hbm, wq_hbm, wk_hbm, wv_hbm, wo_hbm, w1_hbm, w2_hbm, w3_hbm, w4_hbm,
            c_hbm, wmod_hbm, out_hbm,
            x_v, act, wqkv, pre, wo_v, w1_v, w2_v, w3_v, w4_v, c_v, mem_v, mod, fill, sem):
    NSEG, _, D = x_hbm.shape
    _, H, DH = wq_hbm.shape
    M = mem_hbm.shape[0]
    S = NSEG * SEG
    F = w3_hbm.shape[2]
    NO = H // OCT
    ROWS = M + BODY
    NT = NSEG * TAIL
    scale = DH ** -0.5
    body, tail = pl.ds(0, BODY), pl.ds(BODY, TAIL)

    def copy(src, dst, i):
        return pltpu.make_async_copy(src, dst, sem.at[i])

    cp_c = copy(c_hbm, c_v, 0)
    cp_mem = copy(mem_hbm, mem_v, 1)
    cp_xt = copy(x_hbm.at[:, tail, :], x_v.at[:, tail, :], 2)
    cp_early, cp_late = [], [copy(w1_hbm, w1_v, 3), copy(w2_hbm, w2_v, 4)]
    for i, (src, dst, n) in enumerate(((w3_hbm, w3_v, 8 * EARLY), (w4_hbm, w4_v, 32 * EARLY))):
        first, rest = pl.ds(0, n), pl.ds(n, src.shape[1] - n)
        cp_early.append(copy(src.at[:, first, :], dst.at[:, first, :], 5 + 2 * i))
        cp_late.append(copy(src.at[:, rest, :], dst.at[:, rest, :], 6 + 2 * i))

    def cp_wo(n):
        return copy(wo_hbm.at[:, pl.ds(pl.multiple_of(n * LANES, LANES), LANES)], wo_v.at[n], 9 + n)

    def cp_xb(n):
        segs = pl.ds(n * (NSEG * LANES // D), NSEG * LANES // D)
        return copy(x_hbm.at[segs, body, :], x_v.at[segs, body, :], 9 + D // LANES + n)

    def wo_rows(r0, n):
        return jnp.concatenate([wo_v[j, pl.ds(r0, n), :] for j in range(D // LANES)], axis=1)

    def prologue(stage, wmod_v, ht, wsem, msem):
        def cp_mod(j):
            return pltpu.make_async_copy(
                wmod_hbm.at[:, pl.ds(pl.multiple_of(j * D, D), D)], wmod_v.at[j % 4],
                msem.at[j % 4])

        def modulation(j, carry):
            cp_mod(j).wait()

            @pl.when(j == 1)
            def _():
                cp_oct(wq_hbm, 1, 1).start()

            c = c_v[...].astype(F32)
            sc = jnp.broadcast_to(c * jax.nn.sigmoid(c), (16, D)).astype(BF16)
            mod[j] = _dot(sc, wmod_v[j % 4])[:8]
            return carry

        def cp_oct(w_hbm, o, slot):
            return pltpu.make_async_copy(
                w_hbm.at[:, pl.ds(pl.multiple_of(o * OCT, OCT), OCT), :], stage.at[slot],
                wsem.at[slot])

        def relayout(i, b, n):
            w = stage[i % NSTAGE, pl.ds(pl.multiple_of(b * n, n), n), :, :].reshape(n * OCT, DH)
            w = jnp.swapaxes(pltpu.bitcast(w, U32).reshape(n // 2, OCT, DH), 0, 1)
            rows = pl.ds(pl.multiple_of(b * (n // 2), n // 2), n // 2)
            for j in range(OCT // 2):
                even, odd = w[j], w[OCT // 2 + j]
                wqkv[i, rows, pl.ds(2 * j * DH, DH)] = (even & 0xFFFF) | (odd << 16)
                wqkv[i, rows, pl.ds((2 * j + 1) * DH, DH)] = (even >> 16) | ((odd >> 16) << 16)

        cp_oct(wq_hbm, 0, 0).start()
        cp_xt.start()
        cp_c.start()
        cp_mem.start()

        def head_pos(i):
            head = jnp.where(i < 2 * ROWS, i // ROWS, (i - 2 * ROWS) // TAIL)
            pos = jnp.where(i < 2 * ROWS, i % ROWS, ROWS + i % TAIL)
            return head, pos

        hr, pr = head_pos(lax.broadcasted_iota(jnp.int32, fill.shape, 0))
        hc, pc = head_pos(lax.broadcasted_iota(jnp.int32, fill.shape, 1))
        visible = (pr < M) | (pr >= pc)
        fill[...] = jnp.where(hr == hc, jnp.where(visible, 0.0, -1e9 / scale), -jnp.inf)

        def whole_relayout(b, i):
            relayout(i, b, D // OCT)
            return i

        def norm_tail(i, carry):
            segs = pl.ds(i * 8, 8)
            xt = x_v[segs, tail, :].astype(F32).reshape(8 * TAIL, D)
            act[segs, tail, :] = _layernorm(xt).reshape(8, TAIL, D)
            return carry

        cp_xt.wait()
        cp_mod(0).start()
        lax.fori_loop(0, NSEG // 8, norm_tail, 0)
        cp_oct(wq_hbm, 0, 0).wait()
        cp_mod(1).start()
        lax.fori_loop(0, OCT, whole_relayout, 0)
        cp_c.wait()
        lax.fori_loop(0, 2, modulation, 0)
        shift, gain = mod[0][:1], 1.0 + mod[1][:1]
        ht[...] = pltpu.bitcast((act[pl.ds(0, NSEG), tail, :].reshape(NT, D) * gain + shift).astype(BF16), U32)

        def project_tail(i, carry):
            @pl.when(i == 1)
            def _():
                cp_oct(wq_hbm, 1, 1).wait()
                lax.fori_loop(0, OCT, whole_relayout, 1)

            @pl.when((i > 0) & (i + 1 < 3 * NO))
            def _():
                cp_oct(wq_hbm, 0, (i + 1) % NSTAGE).wait()

            for m, w_hbm in enumerate((wq_hbm, wk_hbm, wv_hbm)):
                @pl.when((i + 2) // NO == m)
                def _():
                    cp_oct(w_hbm, (i + 2) % NO, (i + 2) % NSTAGE).start()

            @pl.when((i > 0) & (i <= D // LANES))
            def _():
                cp_wo(i - 1).start()
                cp_xb(i - 1).start()

            @pl.when((i > D // LANES) & (i <= D // LANES + 2))
            def _():
                cp_mod(2 * (i - D // LANES)).start()
                cp_mod(2 * (i - D // LANES) + 1).start()

            @pl.when(i == D // LANES + 2)
            def _():
                for cp in cp_early:
                    cp.start()

            nxt = jnp.where(i == 0, 0, jnp.minimum(i + 1, 3 * NO - 1))
            n = NT // TG
            for j in range(OCT // 2):
                for g in range(TG):
                    lhs = _packed(ht[pl.ds(g * n // 2, n // 2), :])
                    halves = []
                    for h in (2 * j, 2 * j + 1):
                        r = _dot(lhs, _packed(wqkv[i, :, pl.ds(h * DH, DH)]))
                        halves.append(r.reshape(n // TAIL, TAIL, DH))
                        relayout(nxt, h * TG + g, D // (OCT * TG))
                    r = jnp.concatenate(halves, axis=1).reshape(2 * n, DH).astype(BF16)
                    pre[i, pl.ds(g * n, n), pl.ds(j * DH, DH)] = pltpu.bitcast(r, U32)
            return carry

        lax.fori_loop(0, 3 * NO, project_tail, 0)

        lax.fori_loop(2, 6, modulation, 0)

    pl.run_scoped(
        prologue,
        pltpu.VMEM((NSTAGE, D, OCT, DH), BF16),
        pltpu.VMEM((4, D, D), BF16),
        pltpu.VMEM((NT // 2, D), U32),
        pltpu.SemaphoreType.DMA((NSTAGE,)),
        pltpu.SemaphoreType.DMA((4,)),
    )

    def mixer_input(x, att):
        x = x.astype(F32) + mod[2][:1] * att
        h = _layernorm(x) * (1.0 + mod[4][:1]) + mod[3][:1]
        return x, h, _layernorm(h)

    def main(otail, xn, hb, yb, mean, s3, s4, ostage, osem):
        def norm_body(s):
            act[s, body, :] = (_layernorm(x_v[s, body, :].astype(F32)) * (1.0 + mod[1][:1])
                               + mod[0][:1])

        def mixer_input_body(s):
            xn[s, body, :], hb[s, body, :], yb[s] = mixer_input(x_v[s, body, :], act[s, body, :])

        cp_mem.wait()
        for n in range(D // LANES):
            cp_wo(n).wait()
            cp_xb(n).wait()
        for cp in cp_early:
            cp.wait()
        for cp in cp_late:
            cp.start()
        norm_body(0)

        def segment(s, mem):
            @pl.when(s == EARLY)
            def _():
                for cp in cp_late:
                    cp.wait()

            lhs = jnp.concatenate([mem, act[s, body, :]], axis=0).astype(BF16)
            rows = pl.ds(pl.multiple_of(s * TAIL, TAIL), TAIL)
            pad = jnp.zeros((fill.shape[1] - fill.shape[0], DH), BF16)
            qkv, probs, heads = {}, {}, {}
            r4 = jnp.minimum(s * 32, F // 2 - 32)
            side_jobs = (
                [(w3_v, s3, s // 2 * 16, s % 2 * (F // 4) + c) for c in range(0, F // 4, LANES)]
                + [(w4_v, s4, r4 + r, c) for r in (0, 16) for c in range(0, D // 2, LANES)])

            def project(p, m):
                o, j = divmod(p, OCT // 2)
                r = _dot(lhs, _packed(wqkv[m * NO + o, :, pl.ds(2 * j * DH, 2 * DH)]))
                r = r.astype(BF16)
                t = pre[m * NO + o, rows, pl.ds(j * DH, DH)]
                if m == 1 and side_jobs:
                    t = t | _combine_weights(*side_jobs.pop())
                qkv[p, m] = [r[:, :DH], r[:, DH:], _packed(t)]

            def scores(p):
                q = jnp.concatenate(qkv[p, 0], axis=0)
                k = jnp.concatenate(qkv[p, 1] + [pad], axis=0)
                sc = lax.dot_general(q, k, (((1,), (1,)), ((), ())), preferred_element_type=F32)
                f = fill[...]
                sc = jnp.where(f == 0.0, sc, f)
                e = jnp.exp2((sc - jnp.max(sc, axis=-1, keepdims=True))
                             * (scale * math.log2(math.e)))
                inv = pltpu.reciprocal(jnp.sum(e, axis=-1, keepdims=True), full_range=False)
                probs[p] = (e * inv).astype(BF16)

            def values(p, pad):
                ov = _dot(probs[p], jnp.concatenate(qkv[p, 2] + [pad], axis=0))
                heads[p] = [ov[:ROWS].astype(BF16), ov[ROWS:2 * ROWS].astype(BF16)]
                otail[rows, pl.ds(2 * p * DH, DH)] = ov[2 * ROWS:2 * ROWS + TAIL]
                otail[rows, pl.ds((2 * p + 1) * DH, DH)] = ov[2 * ROWS + TAIL:]

            def output(p0, p1):
                o = jnp.concatenate([h for p in range(p0, p1) for h in heads[p]], axis=1)
                return _dot(o, wo_rows(2 * p0 * DH, 2 * (p1 - p0) * DH))

            npair = H // 2
            for p in range(0, npair, 2):
                for pp, m in ((p, 0), (p, 1), (p + 1, 0), (p + 1, 1), (p, 2), (p + 1, 2)):
                    project(pp, m)
                scores(p)
                scores(p + 1)
                if p:
                    values(p - 2, pad)
                    values(p - 1, pad)
                else:
                    mixer_input_body(jnp.maximum(s - 1, 0))
                    norm_body(jnp.minimum(s + 1, NSEG - 1))
            assert not side_jobs
            a = output(0, npair // 2)
            bits = pltpu.bitcast(a[:pad.shape[0] // 2, 2 * DH:3 * DH], U32)
            late_pad = _packed(_zero_after(bits))
            values(npair - 2, late_pad)
            values(npair - 1, late_pad)
            a = a + output(npair // 2, npair)
            act[s, body, :] = a[M:]
            return a[:M]

        lax.fori_loop(0, NSEG, segment, mem_v[...].astype(F32))

        mixer_input_body(NSEG - 1)

        hh = act
        hh[0] = jnp.zeros((SEG, D), F32)
        hh[NSEG + 1] = jnp.zeros((SEG, D), F32)

        def token_mlp(i, carry):
            segs, out = pl.ds(i * SB, SB), pl.ds(1 + i * SB, SB)
            rows = pl.ds(pl.multiple_of(i * SB * TAIL, SB * TAIL), SB * TAIL)
            att = _dot(otail[rows, :].astype(BF16), wo_rows(0, H * DH))
            y = yb[segs].reshape(SB * BODY, D).astype(BF16)
            hh[out, body, :] = _gelu(_dot(y, w1_v[...])).reshape(SB, BODY, D)
            x, h, y = mixer_input(x_v[segs, tail, :].reshape(SB * TAIL, D), att)
            xn[segs, tail, :] = x.reshape(SB, TAIL, D)
            hb[segs, tail, :] = h.reshape(SB, TAIL, D)
            hh[out, tail, :] = _gelu(_dot(y.astype(BF16), w1_v[...])).reshape(SB, TAIL, D)
            return carry

        lax.fori_loop(0, NSEG // SB, token_mlp, 0)

        def shift_mix(i, carry):
            n = RB2 // SEG
            segs = pl.ds(i * n, n)
            g = D // 4
            shifted = [
                hh[pl.ds(i * n, n + 2), :, pl.ds(j * g, g)].reshape(RB2 + 2 * SEG, g)
                [SEG + d:SEG + d + RB2] for j, d in enumerate((-1, 1, -2, 2))]
            hs = _dot(jnp.concatenate(shifted, axis=1).astype(BF16), w2_v[...])
            x1 = hb[segs].reshape(RB2, D) + hs
            hb[segs] = x1.reshape(n, SEG, D)
            mean[pl.ds(pl.multiple_of(i * RB2, RB2), RB2), :] = jnp.broadcast_to(
                jnp.mean(x1, axis=-1, keepdims=True), (RB2, LANES))
            return carry

        lax.fori_loop(0, S // RB2, shift_mix, 0)

        def cp_out(i):
            return pltpu.make_async_copy(
                ostage.at[i % 2], out_hbm.at[pl.ds(pl.multiple_of(i * RB, RB), RB), :],
                osem.at[i % 2])

        def channel_mlp(i, carry):
            @pl.when(i >= 2)
            def _():
                cp_out(i - 2).wait()

            segs = pl.ds(i * (RB // SEG), RB // SEG)
            x1 = hb[segs].reshape(RB, D)
            m = mean[pl.ds(pl.multiple_of(i * RB, RB), RB), :]
            d = x1 - jnp.concatenate([m] * (D // LANES), axis=1)
            z = d * lax.rsqrt(jnp.mean(d * d, axis=-1, keepdims=True) + EPS)
            hr, hd = RB // 2, D // 2
            zs = _strassen_lhs(z[:hr, :hd], z[:hr, hd:], z[hr:, :hd], z[hr:, hd:])
            us = []
            for j in range(0, F // 2, C3):
                quads = _strassen_out(lambda n: _dot(zs[n], _rhs(w3_v, s3, n, j, C3)))
                us.append(_strassen_lhs(*[_gelu(q) for q in quads]))
            us = [jnp.concatenate([u[n] for u in us], axis=1) for n in range(7)]
            for j in range(0, hd, C4):
                quads = _strassen_out(lambda n: _dot(us[n], _rhs(w4_v, s4, n, j, C4)))
                for q, (r, c) in zip(quads, ((0, j), (0, hd + j), (hr, j), (hr, hd + j))):
                    part, cols = pl.ds(i * (RB // SEG) + r // SEG, hr // SEG), pl.ds(c, C4)
                    y = hb[part, :, cols].reshape(hr, C4) + q
                    y = xn[part, :, cols].reshape(hr, C4) + mod[5, :1, cols] * y
                    ostage[i % 2, pl.ds(r, hr), cols] = y.astype(BF16)
            cp_out(i).start()
            return carry

        lax.fori_loop(0, S // RB, channel_mlp, 0)
        cp_out(S // RB - 2).wait()
        cp_out(S // RB - 1).wait()

    pl.run_scoped(
        main,
        pltpu.VMEM((NT, H * DH), F32),
        pltpu.VMEM((NSEG, SEG, D), F32),
        pltpu.VMEM((NSEG, SEG, D), F32),
        pltpu.VMEM((NSEG, BODY, D), F32),
        pltpu.VMEM((S, LANES), F32),
        pltpu.VMEM((5, D // 4, F // 2), U32),
        pltpu.VMEM((5, F // 4, D // 2), U32),
        pltpu.VMEM((2, RB, D), BF16),
        pltpu.SemaphoreType.DMA((2,)),
    )


@jax.jit
def pallas_adaLN_cond__memory_aug_recurrent_mem_tr__mixer_s_mlp__prompt_kernel(
    A_x: jax.Array,
    A_mem0: jax.Array,
    A_Wq: jax.Array,
    A_Wk: jax.Array,
    A_Wv: jax.Array,
    A_Wo: jax.Array,
    A_seg_len: jax.Array,
    B_x: jax.Array,
    B_w1: jax.Array,
    B_w2: jax.Array,
    B_w3: jax.Array,
    B_w4: jax.Array,
    c: jax.Array,
    w_mod: jax.Array,
):
    del A_seg_len, B_x
    B, S, D = A_x.shape
    M = A_mem0.shape[1]
    _, H, DH = A_Wq.shape
    F = B_w3.shape[1]
    assert B == 1 and M == 8 and DH == LANES and S % RB2 == 0

    out = pl.pallas_call(
        _kernel,
        out_shape=jax.ShapeDtypeStruct((S, D), A_x.dtype),
        in_specs=[pl.BlockSpec(memory_space=pl.ANY)] * 12,
        out_specs=pl.BlockSpec(memory_space=pl.ANY),
        scratch_shapes=[
            pltpu.VMEM((S // SEG, SEG, D), BF16),
            pltpu.VMEM((S // SEG + 2, SEG, D), F32),
            pltpu.VMEM((3 * H // OCT, D // 2, OCT * DH), U32),
            pltpu.VMEM((3 * H // OCT, S // SEG * TAIL, OCT * DH // 2), U32),
            pltpu.VMEM((D // LANES, H * DH, LANES), BF16),
            pltpu.VMEM((D, D), BF16),
            pltpu.VMEM((D, D), BF16),
            pltpu.VMEM((2, D // 2, F), BF16),
            pltpu.VMEM((2, F // 2, D), BF16),
            pltpu.VMEM((1, D), BF16),
            pltpu.VMEM((M, D), BF16),
            pltpu.VMEM((6, 8, D), F32),
            pltpu.VMEM((2 * (M + SEG), LANES), F32),
            pltpu.SemaphoreType.DMA((9 + 2 * D // LANES,)),
        ],
        compiler_params=pltpu.CompilerParams(vmem_limit_bytes=127 * 2**20),
    )(A_x.reshape(S // SEG, SEG, D), A_mem0.reshape(M, D), A_Wq, A_Wk, A_Wv,
      A_Wo.reshape(H * DH, D), B_w1, B_w2, B_w3.reshape(2, D // 2, F),
      B_w4.reshape(2, F // 2, D), c, w_mod)
    return out.reshape(B, S, D)
```

```python
import math

import jax
import jax.numpy as jnp
from jax import lax
import jax.experimental.pallas as pl
import jax.experimental.pallas.tpu as pltpu

F32, BF16, U32 = jnp.float32, jnp.bfloat16, jnp.uint32

SEG = 32
TAIL = 8
BODY = SEG - TAIL
OCT = 8
LANES = 128
NSTAGE = 4
SB = 16
RB2 = 512
RB = 128
TG = 4
EPS = 1e-5
EARLY = 6
C4 = 256


def _layernorm(x):
    m = jnp.mean(x, axis=-1, keepdims=True)
    d = x - m
    v = jnp.mean(d * d, axis=-1, keepdims=True)
    return d * lax.rsqrt(v + EPS)


def _gelu(x):
    c1 = math.sqrt(2.0 / math.pi)
    hx = 0.5 * x
    return hx + hx * jnp.tanh(x * (c1 + (c1 * 0.044715) * (x * x)))


def _dot(a, b):
    return jnp.dot(a, b, preferred_element_type=F32)


def _packed(words):
    return pltpu.bitcast(words, BF16)


def _strassen_lhs(top, bottom):
    k = top.shape[1] // 2
    a11, a12, a21, a22 = top[:, :k], top[:, k:], bottom[:, :k], bottom[:, k:]
    return [a.astype(BF16) for a in
            (a11 + a22, a21 + a22, a11, a22, a11 + a12, a21 - a11, a12 - a22)]


def _strassen_rhs(b11, b12, b21, b22):
    return [b.astype(BF16) for b in (b11 + b22, b12 - b22, b21 - b11, b11 + b12, b21 + b22)]


def _zero_after(words):
    return (words >> 16) >> 16


def _combine_weights(w_ref, s_ref, r0, c0):
    half = w_ref.shape[2] // 2
    quads = [w_ref[t, pl.ds(pl.multiple_of(r0, 16), 16),
                   pl.ds(pl.multiple_of(c + c0, LANES), LANES)].astype(F32)
             for t in range(2) for c in (0, half)]
    parts = [pltpu.bitcast(part, U32) for part in _strassen_rhs(*quads)]
    for n, part in enumerate(parts):
        s_ref[n, pl.ds(pl.multiple_of(r0 // 2, 8), 8),
              pl.ds(pl.multiple_of(c0, LANES), LANES)] = part
    return _zero_after(parts[0] | parts[1] | parts[2] | parts[3] | parts[4])


def _rhs(w_ref, s_ref, n, c0, nc, zero=None):
    if n == 1:
        return w_ref[0, :, pl.ds(c0, nc)]
    if n == 4:
        return w_ref[1, :, pl.ds(w_ref.shape[2] // 2 + c0, nc)]
    words = s_ref[n - (n > 1) - (n > 4), :, pl.ds(c0, nc)]
    if zero is not None and n == 0:
        words = jnp.concatenate([words[:8] | zero, words[8:]], axis=0)
    return _packed(words)


def _strassen_out(product):
    p2, p4 = product(1), product(3)
    c21 = p2 + p4
    p1 = product(0)
    c11, c22 = p1 + p4, p1 - p2
    p3 = product(2)
    c22 = c22 + p3
    p5 = product(4)
    c12 = p3 + p5
    c11 = c11 - p5
    c22 = c22 + product(5)
    c11 = c11 + product(6)
    return c11, c12, c21, c22


def _strassen_dot(top, bottom, w_ref, s_ref):
    lhs = _strassen_lhs(top, bottom)
    quads = [_strassen_out(lambda n: _dot(lhs[n], _rhs(w_ref, s_ref, n, c, LANES)))
             for c in range(0, w_ref.shape[2] // 2, LANES)]
    return [jnp.concatenate([q[t + u] for u in range(2) for q in quads], axis=1) for t in (0, 2)]


def _kernel(x_hbm, mem_hbm, wq_hbm, wk_hbm, wv_hbm, wo_hbm, w1_hbm, w2_hbm, w3_hbm, w4_hbm,
            c_hbm, wmod_hbm, out_hbm,
            x_v, act, wqkv, pre, wo_v, w1_v, w2_v, w3_v, w4_v, c_v, mem_v, mod, fill, sem):
    NSEG, _, D = x_hbm.shape
    _, H, DH = wq_hbm.shape
    M = mem_hbm.shape[0]
    S = NSEG * SEG
    F = w3_hbm.shape[2]
    NO = H // OCT
    ROWS = M + BODY
    NT = NSEG * TAIL
    scale = DH ** -0.5
    body, tail = pl.ds(0, BODY), pl.ds(BODY, TAIL)

    def copy(src, dst, i):
        return pltpu.make_async_copy(src, dst, sem.at[i])

    cp_c = copy(c_hbm, c_v, 0)
    cp_mem = copy(mem_hbm, mem_v, 1)
    cp_xt = copy(x_hbm.at[:, tail, :], x_v.at[:, tail, :], 2)
    cp_early, cp_late = [], []
    for i, (src, dst, n) in enumerate(((w1_hbm, w1_v, 8 * EARLY), (w2_hbm, w2_v, 8 * EARLY),
                                       (w3_hbm, w3_v, 8 * EARLY), (w4_hbm, w4_v, 32 * EARLY))):
        first, rest = pl.ds(0, n), pl.ds(n, src.shape[1] - n)
        cp_early.append(copy(src.at[:, first, :], dst.at[:, first, :], 3 + 2 * i))
        cp_late.append(copy(src.at[:, rest, :], dst.at[:, rest, :], 4 + 2 * i))

    def cp_wo(n):
        return copy(wo_hbm.at[:, pl.ds(pl.multiple_of(n * LANES, LANES), LANES)], wo_v.at[n], 11 + n)

    def cp_xb(n):
        segs = pl.ds(n * (NSEG * LANES // D), NSEG * LANES // D)
        return copy(x_hbm.at[segs, body, :], x_v.at[segs, body, :], 11 + D // LANES + n)

    def wo_rows(r0, n):
        return jnp.concatenate([wo_v[j, pl.ds(r0, n), :] for j in range(D // LANES)], axis=1)

    def prologue(stage, wmod_v, ht, wsem, msem):
        def cp_mod(j):
            return pltpu.make_async_copy(
                wmod_hbm.at[:, pl.ds(pl.multiple_of(j * D, D), D)], wmod_v.at[j % 4],
                msem.at[j % 4])

        def modulation(j, carry):
            cp_mod(j).wait()

            @pl.when(j == 1)
            def _():
                cp_oct(wq_hbm, 1, 1).start()

            c = c_v[...].astype(F32)
            sc = jnp.broadcast_to(c * jax.nn.sigmoid(c), (16, D)).astype(BF16)
            mod[j] = _dot(sc, wmod_v[j % 4])[:8]
            return carry

        def cp_oct(w_hbm, o, slot):
            return pltpu.make_async_copy(
                w_hbm.at[:, pl.ds(pl.multiple_of(o * OCT, OCT), OCT), :], stage.at[slot],
                wsem.at[slot])

        def relayout(i, b, n):
            w = stage[i % NSTAGE, pl.ds(pl.multiple_of(b * n, n), n), :, :].reshape(n * OCT, DH)
            w = jnp.swapaxes(pltpu.bitcast(w, U32).reshape(n // 2, OCT, DH), 0, 1)
            rows = pl.ds(pl.multiple_of(b * (n // 2), n // 2), n // 2)
            for j in range(OCT // 2):
                even, odd = w[j], w[OCT // 2 + j]
                wqkv[i, rows, pl.ds(2 * j * DH, DH)] = (even & 0xFFFF) | (odd << 16)
                wqkv[i, rows, pl.ds((2 * j + 1) * DH, DH)] = (even >> 16) | ((odd >> 16) << 16)

        cp_oct(wq_hbm, 0, 0).start()
        cp_xt.start()
        cp_c.start()
        cp_mem.start()

        def head_pos(i):
            head = jnp.where(i < 2 * ROWS, i // ROWS, (i - 2 * ROWS) // TAIL)
            pos = jnp.where(i < 2 * ROWS, i % ROWS, ROWS + i % TAIL)
            return head, pos

        hr, pr = head_pos(lax.broadcasted_iota(jnp.int32, fill.shape, 0))
        hc, pc = head_pos(lax.broadcasted_iota(jnp.int32, fill.shape, 1))
        visible = (pr < M) | (pr >= pc)
        fill[...] = jnp.where(hr == hc, jnp.where(visible, 0.0, -1e9 / scale), -jnp.inf)

        def whole_relayout(b, i):
            relayout(i, b, D // OCT)
            return i

        def norm_tail(i, carry):
            segs = pl.ds(i * 8, 8)
            xt = x_v[segs, tail, :].astype(F32).reshape(8 * TAIL, D)
            act[segs, tail, :] = _layernorm(xt).reshape(8, TAIL, D)
            return carry

        cp_xt.wait()
        cp_mod(0).start()
        lax.fori_loop(0, NSEG // 8, norm_tail, 0)
        cp_oct(wq_hbm, 0, 0).wait()
        cp_mod(1).start()
        lax.fori_loop(0, OCT, whole_relayout, 0)
        cp_c.wait()
        lax.fori_loop(0, 2, modulation, 0)
        shift, gain = mod[0][:1], 1.0 + mod[1][:1]
        ht[...] = pltpu.bitcast((act[pl.ds(0, NSEG), tail, :].reshape(NT, D) * gain + shift).astype(BF16), U32)

        def project_tail(i, carry):
            @pl.when(i == 1)
            def _():
                cp_oct(wq_hbm, 1, 1).wait()
                lax.fori_loop(0, OCT, whole_relayout, 1)

            @pl.when((i > 0) & (i + 1 < 3 * NO))
            def _():
                cp_oct(wq_hbm, 0, (i + 1) % NSTAGE).wait()

            for m, w_hbm in enumerate((wq_hbm, wk_hbm, wv_hbm)):
                @pl.when((i + 2) // NO == m)
                def _():
                    cp_oct(w_hbm, (i + 2) % NO, (i + 2) % NSTAGE).start()

            @pl.when((i > 0) & (i <= D // LANES))
            def _():
                cp_wo(i - 1).start()
                cp_xb(i - 1).start()

            @pl.when((i > D // LANES) & (i <= D // LANES + 2))
            def _():
                cp_mod(2 * (i - D // LANES)).start()
                cp_mod(2 * (i - D // LANES) + 1).start()

            @pl.when(i == D // LANES + 2)
            def _():
                for cp in cp_early:
                    cp.start()

            nxt = jnp.where(i == 0, 0, jnp.minimum(i + 1, 3 * NO - 1))
            n = NT // TG
            for j in range(OCT // 2):
                for g in range(TG):
                    lhs = _packed(ht[pl.ds(g * n // 2, n // 2), :])
                    halves = []
                    for h in (2 * j, 2 * j + 1):
                        r = _dot(lhs, _packed(wqkv[i, :, pl.ds(h * DH, DH)]))
                        halves.append(r.reshape(n // TAIL, TAIL, DH))
                        relayout(nxt, h * TG + g, D // (OCT * TG))
                    r = jnp.concatenate(halves, axis=1).reshape(2 * n, DH).astype(BF16)
                    pre[i, pl.ds(g * n, n), pl.ds(j * DH, DH)] = pltpu.bitcast(r, U32)
            return carry

        lax.fori_loop(0, 3 * NO, project_tail, 0)

        lax.fori_loop(2, 6, modulation, 0)

    pl.run_scoped(
        prologue,
        pltpu.VMEM((NSTAGE, D, OCT, DH), BF16),
        pltpu.VMEM((4, D, D), BF16),
        pltpu.VMEM((NT // 2, D), U32),
        pltpu.SemaphoreType.DMA((NSTAGE,)),
        pltpu.SemaphoreType.DMA((4,)),
    )

    def mixer_input(x, att):
        x = x.astype(F32) + mod[2][:1] * att
        h = _layernorm(x) * (1.0 + mod[4][:1]) + mod[3][:1]
        return x, h, _layernorm(h)

    def main(otail, xn, hb, yb, mean, rstd, s1, s2, s3, s4, ostage, osem):
        def norm_body(s):
            act[s, body, :] = (_layernorm(x_v[s, body, :].astype(F32)) * (1.0 + mod[1][:1])
                               + mod[0][:1])

        def mixer_input_body(s):
            xn[s, body, :], hb[s, body, :], yb[s] = mixer_input(x_v[s, body, :], act[s, body, :])

        cp_mem.wait()
        for n in range(D // LANES):
            cp_wo(n).wait()
            cp_xb(n).wait()
        for cp in cp_early:
            cp.wait()
        for cp in cp_late:
            cp.start()
        norm_body(0)

        def segment(s, mem):
            @pl.when(s == EARLY)
            def _():
                for cp in cp_late:
                    cp.wait()

            lhs = jnp.concatenate([mem, act[s, body, :]], axis=0).astype(BF16)
            rows = pl.ds(pl.multiple_of(s * TAIL, TAIL), TAIL)
            pad = jnp.zeros((fill.shape[1] - fill.shape[0], DH), BF16)
            qkv, probs, heads = {}, {}, {}
            r4 = jnp.minimum(s * 32, F // 2 - 32)
            side_jobs = (
                [(w3_v, s3, s // 2 * 16, s % 2 * (F // 4) + c) for c in range(0, F // 4, LANES)]
                + [(w4_v, s4, r4 + r, c) for r in (0, 16) for c in range(0, D // 2, LANES)]
                + [(w, sw, s // 2 * 16, s % 2 * (D // 4) + c)
                   for w, sw in ((w1_v, s1), (w2_v, s2)) for c in range(0, D // 4, LANES)])

            def project(p, m):
                o, j = divmod(p, OCT // 2)
                r = _dot(lhs, _packed(wqkv[m * NO + o, :, pl.ds(2 * j * DH, 2 * DH)]))
                r = r.astype(BF16)
                t = pre[m * NO + o, rows, pl.ds(j * DH, DH)]
                if (m == 1 or (m == 2 and p % 2)) and side_jobs:
                    t = t | _combine_weights(*side_jobs.pop())
                qkv[p, m] = [r[:, :DH], r[:, DH:], _packed(t)]

            def scores(p):
                q = jnp.concatenate(qkv[p, 0], axis=0)
                k = jnp.concatenate(qkv[p, 1] + [pad], axis=0)
                sc = lax.dot_general(q, k, (((1,), (1,)), ((), ())), preferred_element_type=F32)
                f = fill[...]
                sc = jnp.where(f == 0.0, sc, f)
                e = jnp.exp2((sc - jnp.max(sc, axis=-1, keepdims=True))
                             * (scale * math.log2(math.e)))
                inv = pltpu.reciprocal(jnp.sum(e, axis=-1, keepdims=True), full_range=False)
                probs[p] = (e * inv).astype(BF16)

            def values(p, pad):
                ov = _dot(probs[p], jnp.concatenate(qkv[p, 2] + [pad], axis=0))
                heads[p] = [ov[:ROWS].astype(BF16), ov[ROWS:2 * ROWS].astype(BF16)]
                otail[rows, pl.ds(2 * p * DH, DH)] = ov[2 * ROWS:2 * ROWS + TAIL].astype(BF16)
                otail[rows, pl.ds((2 * p + 1) * DH, DH)] = ov[2 * ROWS + TAIL:].astype(BF16)

            def output(p0, p1):
                o = jnp.concatenate([h for p in range(p0, p1) for h in heads[p]], axis=1)
                return _dot(o, wo_rows(2 * p0 * DH, 2 * (p1 - p0) * DH))

            npair = H // 2
            for p in range(0, npair, 2):
                for pp, m in ((p, 0), (p, 1), (p + 1, 0), (p + 1, 1), (p, 2), (p + 1, 2)):
                    project(pp, m)
                scores(p)
                scores(p + 1)
                if p:
                    values(p - 2, pad)
                    values(p - 1, pad)
                else:
                    mixer_input_body(jnp.maximum(s - 1, 0))
                    norm_body(jnp.minimum(s + 1, NSEG - 1))
            assert not side_jobs
            a = output(0, npair // 2)
            bits = pltpu.bitcast(a[:pad.shape[0] // 2, 2 * DH:3 * DH], U32)
            late_pad = _packed(_zero_after(bits))
            values(npair - 2, late_pad)
            values(npair - 1, late_pad)
            a = a + output(npair // 2, npair)
            act[s, body, :] = a[M:]
            return a[:M]

        lax.fori_loop(0, NSEG, segment, mem_v[...].astype(F32))

        mixer_input_body(NSEG - 1)

        hh = act
        hh[0] = jnp.zeros((SEG, D), F32)
        hh[NSEG + 1] = jnp.zeros((SEG, D), F32)

        def token_mlp(i, carry):
            segs, out = pl.ds(i * SB, SB), pl.ds(1 + i * SB, SB)
            rows = pl.ds(pl.multiple_of(i * SB * TAIL, SB * TAIL), SB * TAIL)
            att = _dot(otail[rows, :], wo_rows(0, H * DH))

            def mlp(y, part):
                n = SB * TAIL // 2
                u = jnp.concatenate(_strassen_dot(y[:n], y[n:], w1_v, s1), axis=0)
                hh[out, part, :] = _gelu(u).reshape(SB, TAIL, D)

            for t in range(0, BODY, TAIL):
                mlp(yb[segs, pl.ds(t, TAIL), :].reshape(SB * TAIL, D), pl.ds(t, TAIL))
            x, h, y = mixer_input(x_v[segs, tail, :].reshape(SB * TAIL, D), att)
            xn[segs, tail, :] = x.reshape(SB, TAIL, D)
            hb[segs, tail, :] = h.reshape(SB, TAIL, D)
            mlp(y, tail)
            return carry

        lax.fori_loop(0, NSEG // SB, token_mlp, 0)

        def shift_mix(i, carry):
            n, g = RB // SEG, D // 4
            for b in range(RB2 // RB):
                blk = i * (RB2 // RB) + b
                shifted = jnp.concatenate([
                    hh[pl.ds(blk * n, n + 2), :, pl.ds(j * g, g)].reshape(RB + 2 * SEG, g)
                    [SEG + d:SEG + d + RB] for j, d in enumerate((-1, 1, -2, 2))], axis=1)
                hs = jnp.concatenate(
                    _strassen_dot(shifted[:RB // 2], shifted[RB // 2:], w2_v, s2), axis=0)
                x1 = hb[pl.ds(blk * n, n)].reshape(RB, D) + hs
                hb[pl.ds(blk * n, n)] = x1.reshape(n, SEG, D)
                mean[pl.ds(pl.multiple_of(blk * RB, RB), RB), :] = jnp.broadcast_to(
                    jnp.mean(x1, axis=-1, keepdims=True), (RB, LANES))
            return carry

        lax.fori_loop(0, S // RB2, shift_mix, 0)

        def cp_out(i):
            return pltpu.make_async_copy(
                ostage.at[i % 2], out_hbm.at[pl.ds(pl.multiple_of(i * RB, RB), RB), :],
                osem.at[i % 2])

        def centred(i):
            m = mean[pl.ds(pl.multiple_of(i * RB, RB), RB), :]
            x1 = hb[pl.ds(i * (RB // SEG), RB // SEG)].reshape(RB, D)
            return x1 - jnp.concatenate([m] * (D // LANES), axis=1)

        def inv_std(i):
            d = centred(i)
            r = lax.rsqrt(jnp.mean(d * d, axis=-1, keepdims=True) + EPS)
            return jnp.broadcast_to(r, (RB, LANES))

        def channel_mlp(i, carry):
            @pl.when(i >= 2)
            def _():
                cp_out(i - 2).wait()

            hr, hd = RB // 2, D // 2
            z = centred(i) * jnp.concatenate([rstd[...]] * (D // LANES), axis=1)
            zs = _strassen_lhs(z[:hr], z[hr:])
            us = []
            for j in range(0, F // 2, LANES):
                zero = None
                if j == F // 4:
                    r = inv_std(jnp.minimum(i + 1, S // RB - 1))
                    rstd[...] = r
                    zero = _zero_after(pltpu.bitcast(jnp.max(r.reshape(RB // 8, 8, LANES), axis=0), U32))
                c11, c12, c21, c22 = [_gelu(q) for q in _strassen_out(
                    lambda n: _dot(zs[n], _rhs(w3_v, s3, n, j, LANES, zero)))]
                us.append(_strassen_lhs(jnp.concatenate([c11, c12], axis=1),
                                        jnp.concatenate([c21, c22], axis=1)))
            us = [jnp.concatenate([u[n] for u in us], axis=1) for n in range(7)]
            for j in range(0, hd, C4):
                quads = _strassen_out(lambda n: _dot(us[n], _rhs(w4_v, s4, n, j, C4)))
                for q, (r, c) in zip(quads, ((0, j), (0, hd + j), (hr, j), (hr, hd + j))):
                    part, cols = pl.ds(i * (RB // SEG) + r // SEG, hr // SEG), pl.ds(c, C4)
                    y = hb[part, :, cols].reshape(hr, C4) + q
                    y = xn[part, :, cols].reshape(hr, C4) + mod[5, :1, cols] * y
                    ostage[i % 2, pl.ds(r, hr), cols] = y.astype(BF16)
            cp_out(i).start()
            return carry

        rstd[...] = inv_std(0)
        lax.fori_loop(0, S // RB, channel_mlp, 0)
        cp_out(S // RB - 2).wait()
        cp_out(S // RB - 1).wait()

    pl.run_scoped(
        main,
        pltpu.VMEM((NT, H * DH), BF16),
        pltpu.VMEM((NSEG, SEG, D), F32),
        pltpu.VMEM((NSEG, SEG, D), F32),
        pltpu.VMEM((NSEG, BODY, D), F32),
        pltpu.VMEM((S, LANES), F32),
        pltpu.VMEM((RB, LANES), F32),
        pltpu.VMEM((5, D // 4, D // 2), U32),
        pltpu.VMEM((5, D // 4, D // 2), U32),
        pltpu.VMEM((5, D // 4, F // 2), U32),
        pltpu.VMEM((5, F // 4, D // 2), U32),
        pltpu.VMEM((2, RB, D), BF16),
        pltpu.SemaphoreType.DMA((2,)),
    )


@jax.jit
def pallas_adaLN_cond__memory_aug_recurrent_mem_tr__mixer_s_mlp__prompt_kernel(
    A_x: jax.Array,
    A_mem0: jax.Array,
    A_Wq: jax.Array,
    A_Wk: jax.Array,
    A_Wv: jax.Array,
    A_Wo: jax.Array,
    A_seg_len: jax.Array,
    B_x: jax.Array,
    B_w1: jax.Array,
    B_w2: jax.Array,
    B_w3: jax.Array,
    B_w4: jax.Array,
    c: jax.Array,
    w_mod: jax.Array,
):
    del A_seg_len, B_x
    B, S, D = A_x.shape
    M = A_mem0.shape[1]
    _, H, DH = A_Wq.shape
    F = B_w3.shape[1]
    assert B == 1 and M == 8 and DH == LANES and S % RB2 == 0

    out = pl.pallas_call(
        _kernel,
        out_shape=jax.ShapeDtypeStruct((S, D), A_x.dtype),
        in_specs=[pl.BlockSpec(memory_space=pl.ANY)] * 12,
        out_specs=pl.BlockSpec(memory_space=pl.ANY),
        scratch_shapes=[
            pltpu.VMEM((S // SEG, SEG, D), BF16),
            pltpu.VMEM((S // SEG + 2, SEG, D), F32),
            pltpu.VMEM((3 * H // OCT, D // 2, OCT * DH), U32),
            pltpu.VMEM((3 * H // OCT, S // SEG * TAIL, OCT * DH // 2), U32),
            pltpu.VMEM((D // LANES, H * DH, LANES), BF16),
            pltpu.VMEM((2, D // 2, D), BF16),
            pltpu.VMEM((2, D // 2, D), BF16),
            pltpu.VMEM((2, D // 2, F), BF16),
            pltpu.VMEM((2, F // 2, D), BF16),
            pltpu.VMEM((1, D), BF16),
            pltpu.VMEM((M, D), BF16),
            pltpu.VMEM((6, 8, D), F32),
            pltpu.VMEM((2 * (M + SEG), LANES), F32),
            pltpu.SemaphoreType.DMA((11 + 2 * D // LANES,)),
        ],
        compiler_params=pltpu.CompilerParams(vmem_limit_bytes=127 * 2**20),
    )(A_x.reshape(S // SEG, SEG, D), A_mem0.reshape(M, D), A_Wq, A_Wk, A_Wv,
      A_Wo.reshape(H * DH, D), B_w1.reshape(2, D // 2, D), B_w2.reshape(2, D // 2, D),
      B_w3.reshape(2, D // 2, F),
      B_w4.reshape(2, F // 2, D), c, w_mod)
    return out.reshape(B, S, D)
```

```python
import math

import jax
import jax.numpy as jnp
from jax import lax
import jax.experimental.pallas as pl
import jax.experimental.pallas.tpu as pltpu

F32, BF16, U32 = jnp.float32, jnp.bfloat16, jnp.uint32

SEG = 32
TAIL = 8
BODY = SEG - TAIL
OCT = 8
LANES = 128
NSTAGE = 4
SB = 16
RB2 = 512
RB = 128
TG = 4
EPS = 1e-5
EARLY = 6
G = 2
COL = 2
C4 = 256


def _layernorm(x):
    m = jnp.mean(x, axis=-1, keepdims=True)
    d = x - m
    v = jnp.mean(d * d, axis=-1, keepdims=True)
    return d * lax.rsqrt(v + EPS)


def _gelu(x):
    c1 = math.sqrt(2.0 / math.pi)
    hx = 0.5 * x
    return hx + hx * jnp.tanh(x * (c1 + (c1 * 0.044715) * (x * x)))


def _dot(a, b):
    return jnp.dot(a, b, preferred_element_type=F32)


def _packed(words):
    return pltpu.bitcast(words, BF16)


def _strassen_lhs(top, bottom):
    k = top.shape[1] // 2
    a11, a12, a21, a22 = top[:, :k], top[:, k:], bottom[:, :k], bottom[:, k:]
    return [a.astype(BF16) for a in
            (a11 + a22, a21 + a22, a11, a22, a11 + a12, a21 - a11, a12 - a22)]


def _strassen_rhs(b11, b12, b21, b22):
    return [b.astype(BF16) for b in (b11 + b22, b12 - b22, b21 - b11, b11 + b12, b21 + b22)]


def _zero_after(words):
    return (words >> 16) >> 16


def _combine_weights(w_ref, s_ref, r0, c0):
    half = w_ref.shape[2] // 2
    quads = [w_ref[t, pl.ds(pl.multiple_of(r0, 16), 16),
                   pl.ds(pl.multiple_of(c + c0, LANES), LANES)].astype(F32)
             for t in range(2) for c in (0, half)]
    parts = [pltpu.bitcast(part, U32) for part in _strassen_rhs(*quads)]
    for n, part in enumerate(parts):
        s_ref[n, pl.ds(pl.multiple_of(r0 // 2, 8), 8),
              pl.ds(pl.multiple_of(c0, LANES), LANES)] = part
    return _zero_after(parts[0] | parts[1] | parts[2] | parts[3] | parts[4])


def _rhs(w_ref, s_ref, n, c0, nc, zero=None):
    if n == 1:
        return w_ref[0, :, pl.ds(c0, nc)]
    if n == 4:
        return w_ref[1, :, pl.ds(w_ref.shape[2] // 2 + c0, nc)]
    words = s_ref[n - (n > 1) - (n > 4), :, pl.ds(c0, nc)]
    if zero is not None and n == 0:
        words = jnp.concatenate([words[:8] | zero, words[8:]], axis=0)
    return _packed(words)


def _strassen_out(product):
    p2, p4 = product(1), product(3)
    c21 = p2 + p4
    p1 = product(0)
    c11, c22 = p1 + p4, p1 - p2
    p3 = product(2)
    c22 = c22 + p3
    p5 = product(4)
    c12 = p3 + p5
    c11 = c11 - p5
    c22 = c22 + product(5)
    c11 = c11 + product(6)
    return c11, c12, c21, c22


def _strassen_dot(top, bottom, w_ref, s_ref):
    lhs = _strassen_lhs(top, bottom)
    quads = [_strassen_out(lambda n: _dot(lhs[n], _rhs(w_ref, s_ref, n, c, LANES)))
             for c in range(0, w_ref.shape[2] // 2, LANES)]
    return [jnp.concatenate([q[t + u] for u in range(2) for q in quads], axis=1) for t in (0, 2)]


def _kernel(x_hbm, mem_hbm, wq_hbm, wk_hbm, wv_hbm, wo_hbm, w1_hbm, w2_hbm, w3_hbm, w4_hbm,
            c_hbm, wmod_hbm, out_hbm,
            x_v, act, wqkv, pre, wo_v, w1_v, w2_v, w3_v, w4_v, c_v, mem_v, mod, fill, sem):
    NSEG, _, D = x_hbm.shape
    _, H, DH = wq_hbm.shape
    M = mem_hbm.shape[0]
    S = NSEG * SEG
    F = w3_hbm.shape[2]
    NO = H // OCT
    ROWS = M + BODY
    NT = NSEG * TAIL
    scale = DH ** -0.5
    body, tail = pl.ds(0, BODY), pl.ds(BODY, TAIL)

    def copy(src, dst, i):
        return pltpu.make_async_copy(src, dst, sem.at[i])

    cp_c = copy(c_hbm, c_v, 0)
    cp_mem = copy(mem_hbm, mem_v, 1)
    cp_xt = copy(x_hbm.at[:, tail, :], x_v.at[:, tail, :], 2)
    cp_early, cp_late = [], []
    for i, (src, dst, n) in enumerate(((w1_hbm, w1_v, 8 * EARLY), (w2_hbm, w2_v, 8 * EARLY),
                                       (w3_hbm, w3_v, 8 * EARLY), (w4_hbm, w4_v, 32 * EARLY))):
        first, rest = pl.ds(0, n), pl.ds(n, src.shape[1] - n)
        cp_early.append(copy(src.at[:, first, :], dst.at[:, first, :], 3 + 2 * i))
        cp_late.append(copy(src.at[:, rest, :], dst.at[:, rest, :], 4 + 2 * i))

    def cp_wo(n):
        return copy(wo_hbm.at[:, pl.ds(pl.multiple_of(n * LANES, LANES), LANES)], wo_v.at[n], 11 + n)

    def cp_xb(n):
        segs = pl.ds(n * (NSEG * LANES // D), NSEG * LANES // D)
        return copy(x_hbm.at[segs, body, :], x_v.at[segs, body, :], 11 + D // LANES + n)

    def wo_rows(r0, n):
        return jnp.concatenate([wo_v[j, pl.ds(r0, n), :] for j in range(D // LANES)], axis=1)

    def prologue(stage, wmod_v, ht, wsem, msem):
        def cp_mod(j):
            return pltpu.make_async_copy(
                wmod_hbm.at[:, pl.ds(pl.multiple_of(j * D, D), D)], wmod_v.at[j % 4],
                msem.at[j % 4])

        def modulation(j, carry):
            cp_mod(j).wait()

            @pl.when(j == 1)
            def _():
                cp_oct(wq_hbm, 1, 1).start()

            c = c_v[...].astype(F32)
            sc = jnp.broadcast_to(c * jax.nn.sigmoid(c), (16, D)).astype(BF16)
            mod[j] = _dot(sc, wmod_v[j % 4])[:8]
            return carry

        def cp_oct(w_hbm, o, slot):
            return pltpu.make_async_copy(
                w_hbm.at[:, pl.ds(pl.multiple_of(o * OCT, OCT), OCT), :], stage.at[slot],
                wsem.at[slot])

        def relayout(i, b, n):
            w = stage[i % NSTAGE, pl.ds(pl.multiple_of(b * n, n), n), :, :].reshape(n * OCT, DH)
            w = jnp.swapaxes(pltpu.bitcast(w, U32).reshape(n // 2, OCT, DH), 0, 1)
            rows = pl.ds(pl.multiple_of(b * (n // 2), n // 2), n // 2)
            for j in range(OCT // 2):
                even, odd = w[j], w[OCT // 2 + j]
                wqkv[i, rows, pl.ds(2 * j * DH, DH)] = (even & 0xFFFF) | (odd << 16)
                wqkv[i, rows, pl.ds((2 * j + 1) * DH, DH)] = (even >> 16) | ((odd >> 16) << 16)

        cp_oct(wq_hbm, 0, 0).start()
        cp_xt.start()
        cp_c.start()
        cp_mem.start()

        def head_pos(i):
            head = jnp.where(i < 2 * ROWS, i // ROWS, (i - 2 * ROWS) // TAIL)
            pos = jnp.where(i < 2 * ROWS, i % ROWS, ROWS + i % TAIL)
            return head, pos

        hr, pr = head_pos(lax.broadcasted_iota(jnp.int32, fill.shape, 0))
        hc, pc = head_pos(lax.broadcasted_iota(jnp.int32, fill.shape, 1))
        visible = (pr < M) | (pr >= pc)
        fill[...] = jnp.where(hr == hc, jnp.where(visible, 0.0, -1e9 / scale), -jnp.inf)

        def whole_relayout(b, i):
            relayout(i, b, D // OCT)
            return i

        def norm_tail(i, carry):
            segs = pl.ds(i * 8, 8)
            xt = x_v[segs, tail, :].astype(F32).reshape(8 * TAIL, D)
            act[segs, tail, :] = _layernorm(xt).reshape(8, TAIL, D)
            return carry

        cp_xt.wait()
        cp_mod(0).start()
        lax.fori_loop(0, NSEG // 8, norm_tail, 0)
        cp_oct(wq_hbm, 0, 0).wait()
        cp_mod(1).start()
        lax.fori_loop(0, OCT, whole_relayout, 0)
        cp_c.wait()
        lax.fori_loop(0, 2, modulation, 0)
        shift, gain = mod[0][:1], 1.0 + mod[1][:1]
        ht[...] = pltpu.bitcast((act[pl.ds(0, NSEG), tail, :].reshape(NT, D) * gain + shift).astype(BF16), U32)

        def project_tail(i, carry):
            @pl.when(i == 1)
            def _():
                cp_oct(wq_hbm, 1, 1).wait()
                lax.fori_loop(0, OCT, whole_relayout, 1)

            @pl.when((i > 0) & (i + 1 < 3 * NO))
            def _():
                cp_oct(wq_hbm, 0, (i + 1) % NSTAGE).wait()

            for m, w_hbm in enumerate((wq_hbm, wk_hbm, wv_hbm)):
                @pl.when((i + 2) // NO == m)
                def _():
                    cp_oct(w_hbm, (i + 2) % NO, (i + 2) % NSTAGE).start()

            @pl.when((i > 0) & (i <= D // LANES))
            def _():
                cp_wo(i - 1).start()
                cp_xb(i - 1).start()

            @pl.when((i > D // LANES) & (i <= D // LANES + 2))
            def _():
                cp_mod(2 * (i - D // LANES)).start()
                cp_mod(2 * (i - D // LANES) + 1).start()

            @pl.when(i == D // LANES + 2)
            def _():
                for cp in cp_early:
                    cp.start()

            nxt = jnp.where(i == 0, 0, jnp.minimum(i + 1, 3 * NO - 1))
            n = NT // TG
            for j in range(OCT // 2):
                for g in range(TG):
                    lhs = _packed(ht[pl.ds(g * n // 2, n // 2), :])
                    halves = []
                    for h in (2 * j, 2 * j + 1):
                        r = _dot(lhs, _packed(wqkv[i, :, pl.ds(h * DH, DH)]))
                        halves.append(r.reshape(n // TAIL, TAIL, DH))
                        relayout(nxt, h * TG + g, D // (OCT * TG))
                    r = jnp.concatenate(halves, axis=1).reshape(2 * n, DH).astype(BF16)
                    pre[i, pl.ds(g * n, n), pl.ds(j * DH, DH)] = pltpu.bitcast(r, U32)
            return carry

        lax.fori_loop(0, 3 * NO, project_tail, 0)

        lax.fori_loop(2, 6, modulation, 0)

    pl.run_scoped(
        prologue,
        pltpu.VMEM((NSTAGE, D, OCT, DH), BF16),
        pltpu.VMEM((4, D, D), BF16),
        pltpu.VMEM((NT // 2, D), U32),
        pltpu.SemaphoreType.DMA((NSTAGE,)),
        pltpu.SemaphoreType.DMA((4,)),
    )

    def mixer_input(x, att):
        x = x.astype(F32) + mod[2][:1] * att
        h = _layernorm(x) * (1.0 + mod[4][:1]) + mod[3][:1]
        return x, h, _layernorm(h)

    def main(otail, xn, hb, yb, mean, rstd, s1, s2, s3, s4, ostage, osem):
        def norm_body(s, t):
            part = pl.ds(t, 8)
            h = _layernorm(x_v[s, part, :].astype(F32)) * (1.0 + mod[1][:1]) + mod[0][:1]
            act[s, part, :] = h
            return _zero_after(pltpu.bitcast(h[:, -LANES:], U32))

        def mixer_input_body(s, t):
            part = pl.ds(t, 8)
            x, h, y = mixer_input(x_v[s, part, :], act[s, part, :])
            xn[s, part, :], hb[s, part, :], yb[s, part, :] = x, h, y
            return _zero_after(pltpu.bitcast(y[:, -LANES:], U32))

        cp_mem.wait()
        for n in range(D // LANES):
            cp_wo(n).wait()
            cp_xb(n).wait()
        for cp in cp_early:
            cp.wait()
        for cp in cp_late:
            cp.start()
        for t in range(0, BODY, 8):
            norm_body(0, t)

        def segment(s, mem):
            lhs = jnp.concatenate([mem, act[s, body, :]], axis=0).astype(BF16)
            rows = pl.ds(pl.multiple_of(s * TAIL, TAIL), TAIL)
            pad = jnp.zeros((fill.shape[1] - fill.shape[0], DH), BF16)
            qkv, probs, heads = {}, {}, {}
            norm_jobs = ([(mixer_input_body, jnp.maximum(s - 1, 0), t) for t in range(0, BODY, 8)]
                         + [(norm_body, jnp.minimum(s + 1, NSEG - 1), t) for t in range(0, BODY, 8)])
            r4 = jnp.minimum(s * 32, F // 2 - 32)
            side_jobs = (
                [(w3_v, s3, s // 2 * 16, s % 2 * (F // 4) + c) for c in range(0, F // 4, LANES)]
                + [(w4_v, s4, r4 + r, c) for r in (0, 16) for c in range(0, D // 2, LANES)]
                + [(w, sw, s // 2 * 16, s % 2 * (D // 4) + c)
                   for w, sw in ((w1_v, s1), (w2_v, s2)) for c in range(0, D // 4, LANES)])

            def project(p, m):
                o, j = divmod(p, OCT // 2)
                r = _dot(lhs, _packed(wqkv[m * NO + o, :, pl.ds(2 * j * DH, 2 * DH)]))
                r = r.astype(BF16)
                t = pre[m * NO + o, rows, pl.ds(j * DH, DH)]
                if (m == 1 or (m == 2 and p % 2)) and side_jobs:
                    t = t | _combine_weights(*side_jobs.pop())
                if m == 0 and p % 2 == 0 and p and norm_jobs:
                    job, *args = norm_jobs.pop(0)
                    t = t | job(*args)
                qkv[p, m] = [r[:, :DH], r[:, DH:], _packed(t)]

            def scores(p):
                q = jnp.concatenate(qkv[p, 0], axis=0)
                k = jnp.concatenate(qkv[p, 1] + [pad], axis=0)
                sc = lax.dot_general(q, k, (((1,), (1,)), ((), ())), preferred_element_type=F32)
                f = fill[...]
                sc = jnp.where(f == 0.0, sc, f)
                e = jnp.exp2((sc - jnp.max(sc, axis=-1, keepdims=True))
                             * (scale * math.log2(math.e)))
                inv = pltpu.reciprocal(jnp.sum(e, axis=-1, keepdims=True), full_range=False)
                probs[p] = (e * inv).astype(BF16)

            def values(p, pad):
                ov = _dot(probs[p], jnp.concatenate(qkv[p, 2] + [pad], axis=0))
                heads[p] = [ov[:ROWS].astype(BF16), ov[ROWS:2 * ROWS].astype(BF16)]
                otail[rows, pl.ds(2 * p * DH, DH)] = ov[2 * ROWS:2 * ROWS + TAIL].astype(BF16)
                otail[rows, pl.ds((2 * p + 1) * DH, DH)] = ov[2 * ROWS + TAIL:].astype(BF16)

            def output(p0, p1):
                o = jnp.concatenate([h for p in range(p0, p1) for h in heads[p]], axis=1)
                return _dot(o, wo_rows(2 * p0 * DH, 2 * (p1 - p0) * DH))

            npair = H // 2
            for p in range(0, npair, G):
                for pp in range(p, p + G):
                    project(pp, 0)
                    project(pp, 1)
                for pp in range(p, p + G):
                    project(pp, 2)
                if p:
                    for pp in range(p - G, p):
                        values(pp, pad)
                for pp in range(p, p + G):
                    scores(pp)
            assert not side_jobs and not norm_jobs
            a = output(0, npair // 2)
            bits = pltpu.bitcast(a[:pad.shape[0] // 2, COL * DH:(COL + 1) * DH], U32)
            late_pad = _packed(_zero_after(bits))
            for pp in range(npair - G, npair):
                values(pp, late_pad)
            a = a + output(npair // 2, npair)
            act[s, body, :] = a[M:]
            return a[:M]

        def two_segments(i, mem):
            @pl.when(2 * i == EARLY)
            def _():
                for cp in cp_late:
                    cp.wait()

            return segment(2 * i + 1, segment(2 * i, mem))

        lax.fori_loop(0, NSEG // 2, two_segments, mem_v[...].astype(F32))

        for t in range(0, BODY, 8):
            mixer_input_body(NSEG - 1, t)

        hh = act
        hh[0] = jnp.zeros((SEG, D), F32)
        hh[NSEG + 1] = jnp.zeros((SEG, D), F32)

        def token_mlp(i, carry):
            segs, out = pl.ds(i * SB, SB), pl.ds(1 + i * SB, SB)
            rows = pl.ds(pl.multiple_of(i * SB * TAIL, SB * TAIL), SB * TAIL)
            att = _dot(otail[rows, :], wo_rows(0, H * DH))

            def mlp(y, part):
                n = SB * TAIL // 2
                u = jnp.concatenate(_strassen_dot(y[:n], y[n:], w1_v, s1), axis=0)
                hh[out, part, :] = _gelu(u).reshape(SB, TAIL, D)

            for t in range(0, BODY, TAIL):
                mlp(yb[segs, pl.ds(t, TAIL), :].reshape(SB * TAIL, D), pl.ds(t, TAIL))
            x, h, y = mixer_input(x_v[segs, tail, :].reshape(SB * TAIL, D), att)
            xn[segs, tail, :] = x.reshape(SB, TAIL, D)
            hb[segs, tail, :] = h.reshape(SB, TAIL, D)
            mlp(y, tail)
            return carry

        lax.fori_loop(0, NSEG // SB, token_mlp, 0)

        def shift_mix(i, carry):
            n, g = RB // SEG, D // 4
            for b in range(RB2 // RB):
                blk = i * (RB2 // RB) + b
                shifted = jnp.concatenate([
                    hh[pl.ds(blk * n, n + 2), :, pl.ds(j * g, g)].reshape(RB + 2 * SEG, g)
                    [SEG + d:SEG + d + RB] for j, d in enumerate((-1, 1, -2, 2))], axis=1)
                hs = jnp.concatenate(
                    _strassen_dot(shifted[:RB // 2], shifted[RB // 2:], w2_v, s2), axis=0)
                x1 = hb[pl.ds(blk * n, n)].reshape(RB, D) + hs
                hb[pl.ds(blk * n, n)] = x1.reshape(n, SEG, D)
                mean[pl.ds(pl.multiple_of(blk * RB, RB), RB), :] = jnp.broadcast_to(
                    jnp.mean(x1, axis=-1, keepdims=True), (RB, LANES))
            return carry

        lax.fori_loop(0, S // RB2, shift_mix, 0)

        def cp_out(i):
            return pltpu.make_async_copy(
                ostage.at[i % 2], out_hbm.at[pl.ds(pl.multiple_of(i * RB, RB), RB), :],
                osem.at[i % 2])

        def centred(i):
            m = mean[pl.ds(pl.multiple_of(i * RB, RB), RB), :]
            x1 = hb[pl.ds(i * (RB // SEG), RB // SEG)].reshape(RB, D)
            return x1 - jnp.concatenate([m] * (D // LANES), axis=1)

        def inv_std(i):
            d = centred(i)
            r = lax.rsqrt(jnp.mean(d * d, axis=-1, keepdims=True) + EPS)
            return jnp.broadcast_to(r, (RB, LANES))

        def channel_mlp(i, carry):
            @pl.when(i >= 2)
            def _():
                cp_out(i - 2).wait()

            hr, hd = RB // 2, D // 2
            z = centred(i) * jnp.concatenate([rstd[...]] * (D // LANES), axis=1)
            zs = _strassen_lhs(z[:hr], z[hr:])
            us = []
            for j in range(0, F // 2, LANES):
                zero = None
                if j == F // 4:
                    r = inv_std(jnp.minimum(i + 1, S // RB - 1))
                    rstd[...] = r
                    zero = _zero_after(pltpu.bitcast(jnp.max(r.reshape(RB // 8, 8, LANES), axis=0), U32))
                c11, c12, c21, c22 = [_gelu(q) for q in _strassen_out(
                    lambda n: _dot(zs[n], _rhs(w3_v, s3, n, j, LANES, zero)))]
                us.append(_strassen_lhs(jnp.concatenate([c11, c12], axis=1),
                                        jnp.concatenate([c21, c22], axis=1)))
            us = [jnp.concatenate([u[n] for u in us], axis=1) for n in range(7)]
            for j in range(0, hd, C4):
                quads = _strassen_out(lambda n: _dot(us[n], _rhs(w4_v, s4, n, j, C4)))
                for q, (r, c) in zip(quads, ((0, j), (0, hd + j), (hr, j), (hr, hd + j))):
                    part, cols = pl.ds(i * (RB // SEG) + r // SEG, hr // SEG), pl.ds(c, C4)
                    y = hb[part, :, cols].reshape(hr, C4) + q
                    y = xn[part, :, cols].reshape(hr, C4) + mod[5, :1, cols] * y
                    ostage[i % 2, pl.ds(r, hr), cols] = y.astype(BF16)
            cp_out(i).start()
            return carry

        rstd[...] = inv_std(0)
        lax.fori_loop(0, S // RB, channel_mlp, 0)
        cp_out(S // RB - 2).wait()
        cp_out(S // RB - 1).wait()

    pl.run_scoped(
        main,
        pltpu.VMEM((NT, H * DH), BF16),
        pltpu.VMEM((NSEG, SEG, D), F32),
        pltpu.VMEM((NSEG, SEG, D), F32),
        pltpu.VMEM((NSEG, BODY, D), F32),
        pltpu.VMEM((S, LANES), F32),
        pltpu.VMEM((RB, LANES), F32),
        pltpu.VMEM((5, D // 4, D // 2), U32),
        pltpu.VMEM((5, D // 4, D // 2), U32),
        pltpu.VMEM((5, D // 4, F // 2), U32),
        pltpu.VMEM((5, F // 4, D // 2), U32),
        pltpu.VMEM((2, RB, D), BF16),
        pltpu.SemaphoreType.DMA((2,)),
    )


@jax.jit
def pallas_adaLN_cond__memory_aug_recurrent_mem_tr__mixer_s_mlp__prompt_kernel(
    A_x: jax.Array,
    A_mem0: jax.Array,
    A_Wq: jax.Array,
    A_Wk: jax.Array,
    A_Wv: jax.Array,
    A_Wo: jax.Array,
    A_seg_len: jax.Array,
    B_x: jax.Array,
    B_w1: jax.Array,
    B_w2: jax.Array,
    B_w3: jax.Array,
    B_w4: jax.Array,
    c: jax.Array,
    w_mod: jax.Array,
):
    del A_seg_len, B_x
    B, S, D = A_x.shape
    M = A_mem0.shape[1]
    _, H, DH = A_Wq.shape
    F = B_w3.shape[1]
    assert B == 1 and M == 8 and DH == LANES and S % RB2 == 0

    out = pl.pallas_call(
        _kernel,
        out_shape=jax.ShapeDtypeStruct((S, D), A_x.dtype),
        in_specs=[pl.BlockSpec(memory_space=pl.ANY)] * 12,
        out_specs=pl.BlockSpec(memory_space=pl.ANY),
        scratch_shapes=[
            pltpu.VMEM((S // SEG, SEG, D), BF16),
            pltpu.VMEM((S // SEG + 2, SEG, D), F32),
            pltpu.VMEM((3 * H // OCT, D // 2, OCT * DH), U32),
            pltpu.VMEM((3 * H // OCT, S // SEG * TAIL, OCT * DH // 2), U32),
            pltpu.VMEM((D // LANES, H * DH, LANES), BF16),
            pltpu.VMEM((2, D // 2, D), BF16),
            pltpu.VMEM((2, D // 2, D), BF16),
            pltpu.VMEM((2, D // 2, F), BF16),
            pltpu.VMEM((2, F // 2, D), BF16),
            pltpu.VMEM((1, D), BF16),
            pltpu.VMEM((M, D), BF16),
            pltpu.VMEM((6, 8, D), F32),
            pltpu.VMEM((2 * (M + SEG), LANES), F32),
            pltpu.SemaphoreType.DMA((11 + 2 * D // LANES,)),
        ],
        compiler_params=pltpu.CompilerParams(vmem_limit_bytes=127 * 2**20),
    )(A_x.reshape(S // SEG, SEG, D), A_mem0.reshape(M, D), A_Wq, A_Wk, A_Wv,
      A_Wo.reshape(H * DH, D), B_w1.reshape(2, D // 2, D), B_w2.reshape(2, D // 2, D),
      B_w3.reshape(2, D // 2, F),
      B_w4.reshape(2, F // 2, D), c, w_mod)
    return out.reshape(B, S, D)
```

```python
import math

import jax
import jax.numpy as jnp
from jax import lax
import jax.experimental.pallas as pl
import jax.experimental.pallas.tpu as pltpu

F32, BF16, U32 = jnp.float32, jnp.bfloat16, jnp.uint32

SEG = 32
TAIL = 8
BODY = SEG - TAIL
OCT = 8
LANES = 128
NSTAGE = 4
SB = 16
RB = 128
RB2 = 512
CB = 256
TG = 4
G = 2
EARLY = 6
EPS = 1e-5


def _layernorm(x):
    m = jnp.mean(x, axis=-1, keepdims=True)
    d = x - m
    v = jnp.mean(d * d, axis=-1, keepdims=True)
    return d * lax.rsqrt(v + EPS)


def _gelu(x):
    c1 = math.sqrt(2.0 / math.pi)
    hx = 0.5 * x
    return hx + hx * jnp.tanh(x * (c1 + (c1 * 0.044715) * (x * x)))


def _dot(a, b):
    return jnp.dot(a, b, preferred_element_type=F32)


def _packed(words):
    return pltpu.bitcast(words, BF16)


def _zero_after(words):
    return (words >> 16) >> 16


def _strassen_lhs(top, bottom):
    k = top.shape[1] // 2
    a11, a12, a21, a22 = top[:, :k], top[:, k:], bottom[:, :k], bottom[:, k:]
    return [a.astype(BF16) for a in
            (a11 + a22, a21 + a22, a11, a22, a11 + a12, a21 - a11, a12 - a22)]


def _strassen_rhs(b11, b12, b21, b22):
    return [b.astype(BF16) for b in (b11 + b22, b12 - b22, b21 - b11, b11 + b12, b21 + b22)]


def _combine_weights(w_ref, s_ref, r0, c0):
    half = w_ref.shape[2] // 2
    quads = [w_ref[t, pl.ds(pl.multiple_of(r0, 16), 16),
                   pl.ds(pl.multiple_of(c + c0, LANES), LANES)].astype(F32)
             for t in range(2) for c in (0, half)]
    parts = [pltpu.bitcast(part, U32) for part in _strassen_rhs(*quads)]
    for n, part in enumerate(parts):
        s_ref[n, pl.ds(pl.multiple_of(r0 // 2, 8), 8),
              pl.ds(pl.multiple_of(c0, LANES), LANES)] = part
    return _zero_after(parts[0] | parts[1] | parts[2] | parts[3] | parts[4])


def _rhs(w_ref, s_ref, n, c0, nc, zero=None):
    if n == 1:
        return w_ref[0, :, pl.ds(c0, nc)]
    if n == 4:
        return w_ref[1, :, pl.ds(w_ref.shape[2] // 2 + c0, nc)]
    words = s_ref[n - (n > 1) - (n > 4), :, pl.ds(c0, nc)]
    if zero is not None and n == 0:
        words = jnp.concatenate([words[:8] | zero, words[8:]], axis=0)
    return _packed(words)


def _strassen_out(product):
    p2, p4 = product(1), product(3)
    c21 = p2 + p4
    p1 = product(0)
    c11, c22 = p1 + p4, p1 - p2
    p3 = product(2)
    c22 = c22 + p3
    p5 = product(4)
    c12 = p3 + p5
    c11 = c11 - p5
    c22 = c22 + product(5)
    c11 = c11 + product(6)
    return c11, c12, c21, c22


def _strassen_dot(top, bottom, w_ref, s_ref):
    lhs = _strassen_lhs(top, bottom)
    quads = [_strassen_out(lambda n: _dot(lhs[n], _rhs(w_ref, s_ref, n, c, LANES)))
             for c in range(0, w_ref.shape[2] // 2, LANES)]
    return [jnp.concatenate([q[t + u] for u in range(2) for q in quads], axis=1) for t in (0, 2)]


def _kernel(x_hbm, mem_hbm, wq_hbm, wk_hbm, wv_hbm, wo_hbm, w1_hbm, w2_hbm, w3_hbm, w4_hbm,
            c_hbm, wmod_hbm, out_hbm,
            x_v, act, wqkv, pre, wo_v, w1_v, w2_v, w3_v, w4_v, c_v, mem_v, mod, fill, sem):
    NSEG, _, D = x_hbm.shape
    _, H, DH = wq_hbm.shape
    M = mem_hbm.shape[0]
    S = NSEG * SEG
    F = w3_hbm.shape[2]
    NO = H // OCT
    ROWS = M + BODY
    NT = NSEG * TAIL
    scale = DH ** -0.5
    body, tail = pl.ds(0, BODY), pl.ds(BODY, TAIL)

    def copy(src, dst, i):
        return pltpu.make_async_copy(src, dst, sem.at[i])

    cp_c = copy(c_hbm, c_v, 0)
    cp_mem = copy(mem_hbm, mem_v, 1)
    cp_xt = copy(x_hbm.at[:, tail, :], x_v.at[:, tail, :], 2)
    cp_early, cp_late = [], []
    for i, (src, dst, n) in enumerate(((w1_hbm, w1_v, 8 * EARLY), (w2_hbm, w2_v, 8 * EARLY),
                                       (w3_hbm, w3_v, 8 * EARLY), (w4_hbm, w4_v, 32 * EARLY))):
        first, rest = pl.ds(0, n), pl.ds(n, src.shape[1] - n)
        cp_early.append(copy(src.at[:, first, :], dst.at[:, first, :], 3 + 2 * i))
        cp_late.append(copy(src.at[:, rest, :], dst.at[:, rest, :], 4 + 2 * i))

    def cp_wo(n):
        cols = pl.ds(pl.multiple_of(n * LANES, LANES), LANES)
        return copy(wo_hbm.at[:, cols], wo_v.at[n], 11 + n)

    def cp_xb(n):
        segs = pl.ds(n * (NSEG * LANES // D), NSEG * LANES // D)
        return copy(x_hbm.at[segs, body, :], x_v.at[segs, body, :], 11 + D // LANES + n)

    def wo_rows(r0, n):
        return jnp.concatenate([wo_v[j, pl.ds(r0, n), :] for j in range(D // LANES)], axis=1)

    def prologue(stage, wmod_v, ht, wsem, msem):
        def cp_mod(j):
            return pltpu.make_async_copy(
                wmod_hbm.at[:, pl.ds(pl.multiple_of(j * D, D), D)], wmod_v.at[j % 4],
                msem.at[j % 4])

        def modulation(j, carry):
            cp_mod(j).wait()

            @pl.when(j == 1)
            def _():
                cp_oct(wq_hbm, 1, 1).start()

            c = c_v[...].astype(F32)
            sc = jnp.broadcast_to(c * jax.nn.sigmoid(c), (16, D)).astype(BF16)
            mod[j] = _dot(sc, wmod_v[j % 4])[:8]
            return carry

        def cp_oct(w_hbm, o, slot):
            return pltpu.make_async_copy(
                w_hbm.at[:, pl.ds(pl.multiple_of(o * OCT, OCT), OCT), :], stage.at[slot],
                wsem.at[slot])

        def relayout(i, b, n):
            w = stage[i % NSTAGE, pl.ds(pl.multiple_of(b * n, n), n), :, :].reshape(n * OCT, DH)
            w = jnp.swapaxes(pltpu.bitcast(w, U32).reshape(n // 2, OCT, DH), 0, 1)
            rows = pl.ds(pl.multiple_of(b * (n // 2), n // 2), n // 2)
            for j in range(OCT // 2):
                even, odd = w[j], w[OCT // 2 + j]
                wqkv[i, rows, pl.ds(2 * j * DH, DH)] = (even & 0xFFFF) | (odd << 16)
                wqkv[i, rows, pl.ds((2 * j + 1) * DH, DH)] = (even >> 16) | ((odd >> 16) << 16)

        cp_oct(wq_hbm, 0, 0).start()
        cp_xt.start()
        cp_c.start()
        cp_mem.start()

        def head_pos(i):
            head = jnp.where(i < 2 * ROWS, i // ROWS, (i - 2 * ROWS) // TAIL)
            pos = jnp.where(i < 2 * ROWS, i % ROWS, ROWS + i % TAIL)
            return head, pos

        hr, pr = head_pos(lax.broadcasted_iota(jnp.int32, fill.shape, 0))
        hc, pc = head_pos(lax.broadcasted_iota(jnp.int32, fill.shape, 1))
        visible = (pr < M) | (pr >= pc)
        fill[...] = jnp.where(hr == hc, jnp.where(visible, 0.0, -1e9 / scale), -jnp.inf)

        def whole_relayout(b, i):
            relayout(i, b, D // OCT)
            return i

        def norm_tail(i, carry):
            segs = pl.ds(i * 8, 8)
            xt = x_v[segs, tail, :].astype(F32).reshape(8 * TAIL, D)
            act[segs, tail, :] = _layernorm(xt).reshape(8, TAIL, D)
            return carry

        cp_xt.wait()
        cp_mod(0).start()
        lax.fori_loop(0, NSEG // 8, norm_tail, 0)
        cp_oct(wq_hbm, 0, 0).wait()
        cp_mod(1).start()
        lax.fori_loop(0, OCT, whole_relayout, 0)
        cp_c.wait()
        lax.fori_loop(0, 2, modulation, 0)
        shift, gain = mod[0][:1], 1.0 + mod[1][:1]
        h = act[pl.ds(0, NSEG), tail, :].reshape(NT, D) * gain + shift
        ht[...] = pltpu.bitcast(h.astype(BF16), U32)

        def project_tail(i, carry):
            @pl.when(i == 1)
            def _():
                cp_oct(wq_hbm, 1, 1).wait()
                lax.fori_loop(0, OCT, whole_relayout, 1)

            @pl.when((i > 0) & (i + 1 < 3 * NO))
            def _():
                cp_oct(wq_hbm, 0, (i + 1) % NSTAGE).wait()

            for m, w_hbm in enumerate((wq_hbm, wk_hbm, wv_hbm)):
                @pl.when((i + 2) // NO == m)
                def _():
                    cp_oct(w_hbm, (i + 2) % NO, (i + 2) % NSTAGE).start()

            @pl.when((i > 0) & (i <= D // LANES))
            def _():
                cp_wo(i - 1).start()
                cp_xb(i - 1).start()

            @pl.when((i > D // LANES) & (i <= D // LANES + 2))
            def _():
                cp_mod(2 * (i - D // LANES)).start()
                cp_mod(2 * (i - D // LANES) + 1).start()

            @pl.when(i == D // LANES + 2)
            def _():
                for cp in cp_early:
                    cp.start()

            nxt = jnp.where(i == 0, 0, jnp.minimum(i + 1, 3 * NO - 1))
            n = NT // TG
            for j in range(OCT // 2):
                for g in range(TG):
                    lhs = _packed(ht[pl.ds(g * n // 2, n // 2), :])
                    halves = []
                    for h in (2 * j, 2 * j + 1):
                        r = _dot(lhs, _packed(wqkv[i, :, pl.ds(h * DH, DH)]))
                        halves.append(r.reshape(n // TAIL, TAIL, DH))
                        relayout(nxt, h * TG + g, D // (OCT * TG))
                    r = jnp.concatenate(halves, axis=1).reshape(2 * n, DH).astype(BF16)
                    pre[i, pl.ds(g * n, n), pl.ds(j * DH, DH)] = pltpu.bitcast(r, U32)
            return carry

        lax.fori_loop(0, 3 * NO, project_tail, 0)
        lax.fori_loop(2, 6, modulation, 0)

    pl.run_scoped(
        prologue,
        pltpu.VMEM((NSTAGE, D, OCT, DH), BF16),
        pltpu.VMEM((4, D, D), BF16),
        pltpu.VMEM((NT // 2, D), U32),
        pltpu.SemaphoreType.DMA((NSTAGE,)),
        pltpu.SemaphoreType.DMA((4,)),
    )

    def mixer_input(x, att):
        x = x.astype(F32) + mod[2][:1] * att
        h = _layernorm(x) * (1.0 + mod[4][:1]) + mod[3][:1]
        return x, h, _layernorm(h)

    def main(otail, xn, hb, yb, mean, rstd, s1, s2, s3, s4, ostage, osem):
        def norm_body(s, t):
            part = pl.ds(t, 8)
            h = _layernorm(x_v[s, part, :].astype(F32)) * (1.0 + mod[1][:1]) + mod[0][:1]
            act[s, part, :] = h
            return _zero_after(pltpu.bitcast(h[:, -LANES:], U32))

        def mixer_input_body(s, t):
            part = pl.ds(t, 8)
            x, h, y = mixer_input(x_v[s, part, :], act[s, part, :])
            xn[s, part, :], hb[s, part, :], yb[s, part, :] = x, h, y
            return _zero_after(pltpu.bitcast(y[:, -LANES:], U32))

        cp_mem.wait()
        for n in range(D // LANES):
            cp_wo(n).wait()
            cp_xb(n).wait()
        for cp in cp_early:
            cp.wait()
        for cp in cp_late:
            cp.start()
        for t in range(0, BODY, 8):
            norm_body(0, t)

        def segment(s, mem):
            lhs = jnp.concatenate([mem, act[s, body, :]], axis=0).astype(BF16)
            rows = pl.ds(pl.multiple_of(s * TAIL, TAIL), TAIL)
            pad = jnp.zeros((fill.shape[1] - fill.shape[0], DH), BF16)
            qkv, probs, heads = {}, {}, {}
            norm_jobs = ([(mixer_input_body, jnp.maximum(s - 1, 0), t) for t in range(0, BODY, 8)]
                         + [(norm_body, jnp.minimum(s + 1, NSEG - 1), t) for t in range(0, BODY, 8)])
            r4 = jnp.minimum(s * 32, F // 2 - 32)
            weight_jobs = (
                [(w3_v, s3, s // 2 * 16, s % 2 * (F // 4) + c) for c in range(0, F // 4, LANES)]
                + [(w4_v, s4, r4 + r, c) for r in (0, 16) for c in range(0, D // 2, LANES)]
                + [(w, sw, s // 2 * 16, s % 2 * (D // 4) + c)
                   for w, sw in ((w1_v, s1), (w2_v, s2)) for c in range(0, D // 4, LANES)])

            def project(p, m):
                o, j = divmod(p, OCT // 2)
                r = _dot(lhs, _packed(wqkv[m * NO + o, :, pl.ds(2 * j * DH, 2 * DH)]))
                r = r.astype(BF16)
                t = pre[m * NO + o, rows, pl.ds(j * DH, DH)]
                if (m == 1 or (m == 2 and p % 2)) and weight_jobs:
                    t = t | _combine_weights(*weight_jobs.pop())
                if m == 0 and p % 2 == 0 and p and norm_jobs:
                    job, *args = norm_jobs.pop(0)
                    t = t | job(*args)
                qkv[p, m] = [r[:, :DH], r[:, DH:], _packed(t)]

            def scores(p):
                q = jnp.concatenate(qkv[p, 0], axis=0)
                k = jnp.concatenate(qkv[p, 1] + [pad], axis=0)
                sc = lax.dot_general(q, k, (((1,), (1,)), ((), ())), preferred_element_type=F32)
                f = fill[...]
                sc = jnp.where(f == 0.0, sc, f)
                e = jnp.exp2((sc - jnp.max(sc, axis=-1, keepdims=True))
                             * (scale * math.log2(math.e)))
                inv = pltpu.reciprocal(jnp.sum(e, axis=-1, keepdims=True), full_range=False)
                probs[p] = (e * inv).astype(BF16)

            def values(p, pad):
                ov = _dot(probs[p], jnp.concatenate(qkv[p, 2] + [pad], axis=0))
                heads[p] = [ov[:ROWS].astype(BF16), ov[ROWS:2 * ROWS].astype(BF16)]
                otail[rows, pl.ds(2 * p * DH, DH)] = ov[2 * ROWS:2 * ROWS + TAIL].astype(BF16)
                otail[rows, pl.ds((2 * p + 1) * DH, DH)] = ov[2 * ROWS + TAIL:].astype(BF16)

            def output(p0, p1):
                o = jnp.concatenate([h for p in range(p0, p1) for h in heads[p]], axis=1)
                return _dot(o, wo_rows(2 * p0 * DH, 2 * (p1 - p0) * DH))

            npair = H // 2
            for p in range(0, npair, G):
                for pp in range(p, p + G):
                    project(pp, 0)
                    project(pp, 1)
                for pp in range(p, p + G):
                    project(pp, 2)
                if p:
                    for pp in range(p - G, p):
                        values(pp, pad)
                for pp in range(p, p + G):
                    scores(pp)
            assert not weight_jobs and not norm_jobs
            a = output(0, npair // 2)
            bits = pltpu.bitcast(a[:pad.shape[0] // 2, 2 * DH:3 * DH], U32)
            late_pad = _packed(_zero_after(bits))
            for pp in range(npair - G, npair):
                values(pp, late_pad)
            a = a + output(npair // 2, npair)
            act[s, body, :] = a[M:]
            return a[:M]

        def two_segments(i, mem):
            @pl.when(2 * i == EARLY)
            def _():
                for cp in cp_late:
                    cp.wait()

            return segment(2 * i + 1, segment(2 * i, mem))

        lax.fori_loop(0, NSEG // 2, two_segments, mem_v[...].astype(F32))

        for t in range(0, BODY, 8):
            mixer_input_body(NSEG - 1, t)

        hh = act
        hh[0] = jnp.zeros((SEG, D), F32)
        hh[NSEG + 1] = jnp.zeros((SEG, D), F32)

        def token_mlp(i, carry):
            segs, out = pl.ds(i * SB, SB), pl.ds(1 + i * SB, SB)
            rows = pl.ds(pl.multiple_of(i * SB * TAIL, SB * TAIL), SB * TAIL)
            att = _dot(otail[rows, :], wo_rows(0, H * DH))

            def mlp(y, part):
                n = SB * TAIL // 2
                u = jnp.concatenate(_strassen_dot(y[:n], y[n:], w1_v, s1), axis=0)
                hh[out, part, :] = _gelu(u).reshape(SB, TAIL, D)

            for t in range(0, BODY, TAIL):
                mlp(yb[segs, pl.ds(t, TAIL), :].reshape(SB * TAIL, D), pl.ds(t, TAIL))
            x, h, y = mixer_input(x_v[segs, tail, :].reshape(SB * TAIL, D), att)
            xn[segs, tail, :] = x.reshape(SB, TAIL, D)
            hb[segs, tail, :] = h.reshape(SB, TAIL, D)
            mlp(y, tail)
            return carry

        lax.fori_loop(0, NSEG // SB, token_mlp, 0)

        def shift_mix(i, carry):
            n, g = RB // SEG, D // 4
            for b in range(RB2 // RB):
                blk = i * (RB2 // RB) + b
                shifted = jnp.concatenate([
                    hh[pl.ds(blk * n, n + 2), :, pl.ds(j * g, g)].reshape(RB + 2 * SEG, g)
                    [SEG + d:SEG + d + RB] for j, d in enumerate((-1, 1, -2, 2))], axis=1)
                hs = jnp.concatenate(
                    _strassen_dot(shifted[:RB // 2], shifted[RB // 2:], w2_v, s2), axis=0)
                x1 = hb[pl.ds(blk * n, n)].reshape(RB, D) + hs
                hb[pl.ds(blk * n, n)] = x1.reshape(n, SEG, D)
                mean[pl.ds(pl.multiple_of(blk * RB, RB), RB), :] = jnp.broadcast_to(
                    jnp.mean(x1, axis=-1, keepdims=True), (RB, LANES))
            return carry

        lax.fori_loop(0, S // RB2, shift_mix, 0)

        def cp_out(i):
            return pltpu.make_async_copy(
                ostage.at[i % 2], out_hbm.at[pl.ds(pl.multiple_of(i * RB, RB), RB), :],
                osem.at[i % 2])

        def centred(i):
            m = mean[pl.ds(pl.multiple_of(i * RB, RB), RB), :]
            x1 = hb[pl.ds(i * (RB // SEG), RB // SEG)].reshape(RB, D)
            return x1 - jnp.concatenate([m] * (D // LANES), axis=1)

        def inv_std(i):
            d = centred(i)
            r = lax.rsqrt(jnp.mean(d * d, axis=-1, keepdims=True) + EPS)
            return jnp.broadcast_to(r, (RB, LANES))

        def channel_mlp(i, carry):
            @pl.when(i >= 2)
            def _():
                cp_out(i - 2).wait()

            hr, hd = RB // 2, D // 2
            z = centred(i) * jnp.concatenate([rstd[...]] * (D // LANES), axis=1)
            zs = _strassen_lhs(z[:hr], z[hr:])
            us = []
            for j in range(0, F // 2, LANES):
                zero = None
                if j == F // 4:
                    r = inv_std(jnp.minimum(i + 1, S // RB - 1))
                    rstd[...] = r
                    r = jnp.max(r.reshape(RB // 8, 8, LANES), axis=0)
                    zero = _zero_after(pltpu.bitcast(r, U32))
                c11, c12, c21, c22 = [_gelu(q) for q in _strassen_out(
                    lambda n: _dot(zs[n], _rhs(w3_v, s3, n, j, LANES, zero)))]
                us.append(_strassen_lhs(jnp.concatenate([c11, c12], axis=1),
                                        jnp.concatenate([c21, c22], axis=1)))
            us = [jnp.concatenate([u[n] for u in us], axis=1) for n in range(7)]
            for j in range(0, hd, CB):
                quads = _strassen_out(lambda n: _dot(us[n], _rhs(w4_v, s4, n, j, CB)))
                for q, (r, c) in zip(quads, ((0, j), (0, hd + j), (hr, j), (hr, hd + j))):
                    part, cols = pl.ds(i * (RB // SEG) + r // SEG, hr // SEG), pl.ds(c, CB)
                    y = hb[part, :, cols].reshape(hr, CB) + q
                    y = xn[part, :, cols].reshape(hr, CB) + mod[5, :1, cols] * y
                    ostage[i % 2, pl.ds(r, hr), cols] = y.astype(BF16)
            cp_out(i).start()
            return carry

        rstd[...] = inv_std(0)
        lax.fori_loop(0, S // RB, channel_mlp, 0)
        cp_out(S // RB - 2).wait()
        cp_out(S // RB - 1).wait()

    pl.run_scoped(
        main,
        pltpu.VMEM((NT, H * DH), BF16),
        pltpu.VMEM((NSEG, SEG, D), F32),
        pltpu.VMEM((NSEG, SEG, D), F32),
        pltpu.VMEM((NSEG, BODY, D), F32),
        pltpu.VMEM((S, LANES), F32),
        pltpu.VMEM((RB, LANES), F32),
        pltpu.VMEM((5, D // 4, D // 2), U32),
        pltpu.VMEM((5, D // 4, D // 2), U32),
        pltpu.VMEM((5, D // 4, F // 2), U32),
        pltpu.VMEM((5, F // 4, D // 2), U32),
        pltpu.VMEM((2, RB, D), BF16),
        pltpu.SemaphoreType.DMA((2,)),
    )


@jax.jit
def pallas_adaLN_cond__memory_aug_recurrent_mem_tr__mixer_s_mlp__prompt_kernel(
    A_x: jax.Array,
    A_mem0: jax.Array,
    A_Wq: jax.Array,
    A_Wk: jax.Array,
    A_Wv: jax.Array,
    A_Wo: jax.Array,
    A_seg_len: jax.Array,
    B_x: jax.Array,
    B_w1: jax.Array,
    B_w2: jax.Array,
    B_w3: jax.Array,
    B_w4: jax.Array,
    c: jax.Array,
    w_mod: jax.Array,
):
    del A_seg_len, B_x
    B, S, D = A_x.shape
    M = A_mem0.shape[1]
    _, H, DH = A_Wq.shape
    F = B_w3.shape[1]
    assert (B, S, D, M, H, DH, F) == (1, 2048, 1024, 8, 32, LANES, 3584)

    out = pl.pallas_call(
        _kernel,
        out_shape=jax.ShapeDtypeStruct((S, D), A_x.dtype),
        in_specs=[pl.BlockSpec(memory_space=pl.ANY)] * 12,
        out_specs=pl.BlockSpec(memory_space=pl.ANY),
        scratch_shapes=[
            pltpu.VMEM((S // SEG, SEG, D), BF16),
            pltpu.VMEM((S // SEG + 2, SEG, D), F32),
            pltpu.VMEM((3 * H // OCT, D // 2, OCT * DH), U32),
            pltpu.VMEM((3 * H // OCT, S // SEG * TAIL, OCT * DH // 2), U32),
            pltpu.VMEM((D // LANES, H * DH, LANES), BF16),
            pltpu.VMEM((2, D // 2, D), BF16),
            pltpu.VMEM((2, D // 2, D), BF16),
            pltpu.VMEM((2, D // 2, F), BF16),
            pltpu.VMEM((2, F // 2, D), BF16),
            pltpu.VMEM((1, D), BF16),
            pltpu.VMEM((M, D), BF16),
            pltpu.VMEM((6, 8, D), F32),
            pltpu.VMEM((2 * (M + SEG), LANES), F32),
            pltpu.SemaphoreType.DMA((11 + 2 * D // LANES,)),
        ],
        compiler_params=pltpu.CompilerParams(vmem_limit_bytes=127 * 2**20),
    )(A_x.reshape(S // SEG, SEG, D), A_mem0.reshape(M, D), A_Wq, A_Wk, A_Wv,
      A_Wo.reshape(H * DH, D), B_w1.reshape(2, D // 2, D), B_w2.reshape(2, D // 2, D),
      B_w3.reshape(2, D // 2, F), B_w4.reshape(2, F // 2, D), c, w_mod)
    return out.reshape(B, S, D)
```
